```python
import os as _os
_os.environ.setdefault("JAX_PLATFORMS", "cpu")
import jax
import jax.numpy as jnp

def _softmax(x, axis=-1):
    return jax.nn.softmax(x, axis=axis)
def _gelu(x):
    return jax.nn.gelu(x, approximate=True)
def _silu(x):
    return jax.nn.silu(x)
def _sigmoid(x):
    return jax.nn.sigmoid(x)
def _layernorm(x, axis=-1, eps=1e-5):
    m = jnp.mean(x, axis=axis, keepdims=True)
    v = jnp.var(x, axis=axis, keepdims=True)
    return (x - m) / jnp.sqrt(v + eps)
def _scatter_add(tgt, idx, src, axis=0):
    return tgt.at[idx].add(src)
def _segment_sum(src, seg, n):
    return jax.ops.segment_sum(src, seg, n)
class _Rng:
    def __init__(self, key):
        self._k = key
    def _next(self):
        self._k, sub = jax.random.split(self._k)
        return sub
    def normal(self, shape):
        return jax.random.normal(self._next(), shape, dtype=jnp.bfloat16)
    def randint(self, lo, hi, shape):
        return jax.random.randint(self._next(), shape, lo, hi, dtype=jnp.int32)
    def uniform(self, shape, lo=0.0, hi=1.0):
        return jax.random.uniform(self._next(), shape, jnp.bfloat16, lo, hi)
    def permutation(self, n):
        return jax.random.permutation(self._next(), n)


kernel_name = 'sequential_preLN__linear_kernel_hedgehog__geglu_ffn__prompt'

def setup_inputs():
    _rng = _Rng(jax.random.key(int.from_bytes(__import__("os").urandom(4), "little")))
    _w = (lambda a: (lambda t: t.astype(jnp.bfloat16) if jnp.issubdtype(t.dtype, jnp.floating) else t)(jnp.asarray(a)))
    def _A_setup():
        B, S, D, H = 1, 2048, 640, 32
        Dh = D // H
        return {
            "x": _w((lambda *s: _rng.normal(s) * 0.05)(B, S, D)),
            "wqkv": _w((lambda *s: _rng.normal(s) * 0.2)(D, 3 * D)),
            "w_phi": _w((lambda *s: _rng.normal(s) * 0.2)(H, Dh, Dh) * (Dh ** -0.5)),
            "wo": _w((lambda *s: _rng.normal(s) * 0.05)(D, D)),
        }
    _A_in = _A_setup()

    def _B_setup():
        B, S, D, F = 1, 2048, 640, 1536
        return {
            "x": _w((lambda *s: _rng.normal(s) * 0.05)(B, S, D)),
            "w_gate": _w((lambda *s: _rng.normal(s) * 0.05)(D, F)),
            "w_up": _w((lambda *s: _rng.normal(s) * 0.05)(D, F)),
            "w_down": _w((lambda *s: _rng.normal(s) * 0.05)(F, D)),
        }
    _B_in = _B_setup()

    return {
        "A_x": _A_in["x"],
        "A_wqkv": _A_in["wqkv"],
        "A_w_phi": _A_in["w_phi"],
        "A_wo": _A_in["wo"],
        "B_x": _B_in["x"],
        "B_w_gate": _B_in["w_gate"],
        "B_w_up": _B_in["w_up"],
        "B_w_down": _B_in["w_down"],
    }

def reference(A_x, A_wqkv, A_w_phi, A_wo, B_x, B_w_gate, B_w_up, B_w_down):
    def _A_ref(x, wqkv, w_phi, wo):
        B, S, D = x.shape
        H = 32; Dh = D // H
        qkv = (lambda x, *d: x.transpose(*d))((x @ wqkv).reshape(B, S, 3, H, Dh), 2, 0, 3, 1, 4)
        q, k, v = qkv[0], qkv[1], qkv[2]
        pq = jnp.einsum("bhsd,hdf->bhsf", q, w_phi)
        pk = jnp.einsum("bhsd,hdf->bhsf", k, w_phi)
        phi_q = jnp.concatenate([_softmax(pq, axis=-1), _softmax(-pq, axis=-1)], axis=-1)
        phi_k = jnp.concatenate([_softmax(pk, axis=-1), _softmax(-pk, axis=-1)], axis=-1)
        kv = jnp.einsum("bhsf,bhsd->bhfd", phi_k, v)
        z  = jnp.einsum("bhsf->bhf", phi_k)
        num = jnp.einsum("bhqf,bhfd->bhqd", phi_q, kv)
        den = jnp.einsum("bhqf,bhf->bhq", phi_q, z)[..., None] + 1e-6
        o = num / den
        return (lambda x, *d: x.transpose(*d))(o, 0, 2, 1, 3).reshape(B, S, D) @ wo

    def _B_ref(x, w_gate, w_up, w_down):
        return (_gelu(x @ w_gate) * (x @ w_up)) @ w_down

    x = A_x
    h = x + _A_ref(_layernorm(x, axis=-1), A_wqkv, A_w_phi, A_wo)
    h2 = h + _B_ref(_layernorm(h, axis=-1), B_w_gate, B_w_up, B_w_down)
    return h2
```

```python
import functools
import jax
import jax.numpy as jnp
from jax import lax
import jax.experimental.pallas as pl
import jax.experimental.pallas.tpu as pltpu

S, D, H, DH, F = 2048, 640, 32, 20, 1536
NG = H // 2
GR = 2 * DH
LOG2E = 1.4426950408889634
NT = (((1,), (1,)), ((), ()))
TN = (((0,), (0,)), ((), ()))
f32 = jnp.float32
bf16 = jnp.bfloat16
u32 = jnp.uint32
SB = 256
NSUB = S // SB


def _layernorm(x):
    m = jnp.mean(x, axis=-1, keepdims=True)
    xc = x - m
    v = jnp.mean(xc * xc, axis=-1, keepdims=True)
    return xc * lax.rsqrt(v + 1e-5)


def _recip(x):
    r = pl.reciprocal(x, approx=True)
    return r * (2.0 - x * r)


def _fold8(x, op):
    x = op(x, pltpu.roll(x, 2, 0))
    return op(x, pltpu.roll(x, 4, 0))


def _dual_softmax(p):
    T = p.shape[1]
    p3 = p.reshape(5, 8, T)
    mx = _fold8(jnp.max(p3, axis=0), jnp.maximum)
    mn = _fold8(jnp.min(p3, axis=0), jnp.minimum)
    ep = jnp.exp2(p3 - mx[None])
    en = jnp.exp2(mn[None] - p3)
    rp = _recip(_fold8(jnp.sum(ep, axis=0), jnp.add))
    rn = _recip(_fold8(jnp.sum(en, axis=0), jnp.add))
    phi = jnp.concatenate([ep * rp[None], en * rn[None]], axis=0)
    return phi.reshape(2 * GR, T).astype(bf16)


def _pk(val):
    return pltpu.bitcast(val, u32)


def _upk(val):
    return pltpu.bitcast(val, bf16)


def _half(off):
    if isinstance(off, int):
        return off // 2
    return pl.multiple_of(off // 2, 8)


def _kernel(x_hbm, wqkv_hbm, wphi_hbm, wo_hbm, wg_hbm, wu_hbm, wd_hbm, out_hbm,
            x_v, wqkv_v, wphi_v, wo_v, wg_v, wu_v, wd_v, out_v,
            xn_v, wall, phiq, phik_s, vext_s, kvt, lmat, x_sem, w_sem, o_sem, *, T2, SB2, SBO, PS, NLOOP):
    NB2 = S // T2

    xchunks = [(0, SB), (SB, SB), (2 * SB, S - 2 * SB)]
    x_h32 = x_hbm.bitcast(u32)
    wqkv_h32 = wqkv_hbm.bitcast(u32)

    def x_copy(i):
        o, n = xchunks[i]
        return pltpu.make_async_copy(x_h32.at[pl.ds(o // 2, n // 2)], x_v.at[pl.ds(o // 2, n // 2)], x_sem.at[i])

    def wqkv_copy(j):
        return pltpu.make_async_copy(wqkv_h32.at[:, pl.ds(j * D, D)], wqkv_v.at[:, pl.ds(j * D, D)], w_sem.at[j])

    def other(n):
        src, dst = ((wo_hbm, wo_v), (wg_hbm, wg_v), (wu_hbm, wu_v), (wd_hbm, wd_v), (wphi_hbm, wphi_v))[n]
        if n < 4:
            src = src.bitcast(u32)
        return pltpu.make_async_copy(src, dst, w_sem.at[3 + n])

    def out_copy(i):
        return pltpu.make_async_copy(out_v.at[pl.ds(i * SBO, SBO)], out_hbm.at[pl.ds(i * SBO, SBO)], o_sem.at[i])

    other(4).start()
    x_copy(0).start()
    wqkv_copy(2).start()
    wqkv_copy(1).start()
    x_copy(1).start()
    wqkv_copy(0).start()
    x_copy(2).start()

    hh = lax.broadcasted_iota(jnp.int32, (H, D), 0)
    cc = lax.broadcasted_iota(jnp.int32, (H, D), 1)
    inhead = (cc >= hh * DH) & (cc < hh * DH + DH)
    expand = jnp.where(inhead, 1.0, 0.0).astype(bf16)
    dcol = jnp.sum(jnp.where(inhead, cc - hh * DH, 0), axis=0, keepdims=True)
    r = lax.broadcasted_iota(jnp.int32, (2 * GR, DH), 0)
    j = lax.broadcasted_iota(jnp.int32, (2 * GR, DH), 1)
    rr = jnp.where(r >= GR, r - GR, r)
    a0 = jnp.where((rr >> 1) == j, 1.0, 0.0).astype(bf16)
    other(4).wait()
    t0 = jnp.zeros((DH, D), f32)
    for d in range(DH):
        z = jnp.dot(wphi_v[d], expand, preferred_element_type=f32)
        t0 = jnp.where(dcol == d, z, t0)
    t0 = jnp.dot(a0, t0.astype(bf16), preferred_element_type=f32)
    r = lax.broadcasted_iota(jnp.int32, (2 * GR, D), 0)
    c = lax.broadcasted_iota(jnp.int32, (2 * GR, D), 1)
    hl = jnp.where(r >= GR, 2, 0) + (r & 1)
    pts = []
    for p in range(NG // 2):
        lo = (80 * p) // 128 * 128
        hi = -(-(80 * p + 80) // 128) * 128
        start = (4 * p + hl) * DH
        m = (c >= start) & (c < start + DH)
        pts.append((lo, hi, jnp.where(m, t0, 0.0)[:, lo:hi].astype(bf16)))

    def fold(j):
        for p, (lo, hi, pt) in enumerate(pts):
            w = _upk(wqkv_v[:, j * D + lo:j * D + hi])
            res = lax.dot_general(pt, w, NT, preferred_element_type=f32) * LOG2E
            wall[(j * D + 80 * p) // 2:(j * D + 80 * p + 80) // 2, :] = _pk(res.astype(bf16))

    def ldx(off, n):
        return _upk(x_v[pl.ds(_half(off), n // 2), :]).astype(f32)

    def ln1(off):
        return _layernorm(ldx(off, SB)).astype(bf16)

    def proj(j, xn):
        n = D // PS
        return jnp.concatenate(
            [lax.dot_general(_upk(wall[(j * D + u * n) // 2:(j * D + (u + 1) * n) // 2, :]), xn, NT,
                             preferred_element_type=f32) for u in range(PS)], axis=0)

    def sq(pq, off):
        for g in range(NG):
            phiq[40 * g:40 * (g + 1), pl.ds(off, SB)] = _pk(_dual_softmax(pq[GR * g:GR * (g + 1)]))

    def sk(pk, slot):
        for g in range(NG):
            phik_s[40 * g:40 * (g + 1), slot * SB:(slot + 1) * SB] = _pk(_dual_softmax(pk[GR * g:GR * (g + 1)]))

    def sv(pv, slot):
        ones = jnp.ones((8, SB), f32)
        for g in range(NG):
            vext_s[24 * g:24 * (g + 1), slot * SB:(slot + 1) * SB] = _pk(
                jnp.concatenate([pv[GR * g:GR * (g + 1)], ones], axis=0).astype(bf16))

    def kv(slot, first=False, nslot=1):
        for g in range(NG):
            upd = lax.dot_general(_upk(vext_s[24 * g:24 * (g + 1), slot * SB:(slot + nslot) * SB]),
                                  _upk(phik_s[40 * g:40 * (g + 1), slot * SB:(slot + nslot) * SB]),
                                  NT, preferred_element_type=f32)
            if first:
                kvt[48 * g:48 * (g + 1), :] = upd
            else:
                kvt[48 * g:48 * (g + 1), :] += upd

    def pair(xna, off, noff, extra=None, extra_kv=None):
        pka = proj(1, xna)
        ex = [(proj(0, xn), o) for xn, o in (extra or [])]
        pqa = proj(0, xna)
        pva = proj(2, xna)
        sk(pka, 0)
        for pq, o in ex:
            sq(pq, o)
        sq(pqa, off)
        sv(pva, 0)
        if noff is not None:
            xn_v[...] = _pk(ln1(noff))
        xnb = ln1(off + SB)
        pkb = proj(1, xnb)
        pqb = proj(0, xnb)
        pvb = proj(2, xnb)
        sk(pkb, 1)
        sq(pqb, off + SB)
        sv(pvb, 1)
        if extra_kv is not None:
            extra_kv()
        kv(0)
        kv(1)

    x_copy(0).wait()
    xn0 = ln1(0)
    wqkv_copy(2).wait()
    wvt = _upk(wqkv_v[:, 2 * D:3 * D]).T
    wall[D:3 * D // 2, :] = _pk(wvt)
    pv0 = jnp.concatenate([lax.dot_general(wvt[u * 320:(u + 1) * 320], xn0, NT, preferred_element_type=f32)
                           for u in range(2)], axis=0)
    sv(pv0, 0)
    wqkv_copy(1).wait()
    x_copy(1).wait()
    fold(1)
    xn1 = ln1(SB)
    pk1 = proj(1, xn1)
    pk0 = proj(1, xn0)
    pv1 = proj(2, xn1)
    sk(pk1, 2)
    sk(pk0, 0)
    sv(pv1, 2)
    kv(0, first=True)
    wqkv_copy(0).wait()
    x_copy(2).wait()
    for n in range(4):
        other(n).start()
    fold(0)
    nstraight = 3 - NLOOP
    for q in range(nstraight):
        off = (2 + 2 * q) * SB
        last = q == nstraight - 1
        pair(ln1(off), off, off + 2 * SB if (last and NLOOP) else None,
             [(xn0, 0), (xn1, SB)] if q == 0 else None, (lambda: kv(2)) if q == 0 else None)

    def phase1(i, carry):
        off = pl.multiple_of((2 + 2 * nstraight + i * 2) * SB, SB)
        noff = pl.multiple_of(jnp.minimum(4 + 2 * nstraight + i * 2, NSUB - 1) * SB, SB)
        pair(_upk(xn_v[...]), off, noff)
        return carry

    if NLOOP:
        lax.fori_loop(0, NLOOP, phase1, 0)

    r = lax.broadcasted_iota(jnp.int32, (48, 80), 0)
    c = lax.broadcasted_iota(jnp.int32, (48, 80), 1)
    rh = jnp.where(r < DH, 0, jnp.where(r < GR, 1, jnp.where(r < GR + 4, 0, 1)))
    m = rh == (c & 1)
    for g in range(NG):
        lmat[24 * g:24 * (g + 1), :] = _pk(jnp.where(m, kvt[48 * g:48 * (g + 1), :], 0.0).astype(bf16))

    for n in range(4):
        other(n).wait()

    def phase2(i, carry):
        off = pl.multiple_of(i * T2, T2)
        n = T2 // SB2
        sub = lax.broadcasted_iota(jnp.int32, (8, SB2), 0)
        ots = []
        for s in range(n):
            parts = []
            for g in range(NG):
                ph = _upk(phiq[40 * g:40 * (g + 1), pl.ds(off + s * SB2, SB2)])
                og = jnp.dot(_upk(lmat[24 * g:24 * (g + 1), :]), ph, preferred_element_type=f32)
                rc = _recip(og[40:48] + 1e-6)
                rr = pltpu.roll(rc, 4, 0)
                r0 = jnp.where(sub < 4, rc, rr)
                r1 = jnp.where(sub < 4, rr, rc)
                parts += [og[0:8] * r0, og[8:16] * r0, og[16:24] * rc, og[24:32] * r1, og[32:40] * r1]
            ots.append(jnp.concatenate(parts, axis=0).astype(bf16))
        hs = []
        for s in range(n):
            attn = lax.dot_general(ots[s], _upk(wo_v[...]), TN, preferred_element_type=f32)
            h = ldx(off + s * SB2, SB2) + attn
            hs.append((h, _layernorm(h).astype(bf16)))
        acts = []
        for s in range(n):
            hn = hs[s][1]
            gate = jnp.dot(hn, _upk(wg_v[...]), preferred_element_type=f32)
            up = jnp.dot(hn, _upk(wu_v[...]), preferred_element_type=f32)
            acts.append((jax.nn.gelu(gate, approximate=True) * up).astype(bf16))
        for s in range(n):
            for u in range(SB2 // SBO):
                y = hs[s][0][u * SBO:(u + 1) * SBO] + jnp.dot(acts[s][u * SBO:(u + 1) * SBO], _upk(wd_v[...]),
                                                              preferred_element_type=f32)
                out_v[pl.ds(off + s * SB2 + u * SBO, SBO), :] = y.astype(bf16)
                out_copy(i * (T2 // SBO) + s * (SB2 // SBO) + u).start()
        return carry

    lax.fori_loop(0, NB2, phase2, 0)
    for i in range(S // SBO):
        out_copy(i).wait()


def _compiler_params():
    try:
        return pltpu.CompilerParams(vmem_limit_bytes=100 * 1024 * 1024, disable_bounds_checks=True,
                                    disable_semaphore_checks=True)
    except TypeError:
        return pltpu.CompilerParams(vmem_limit_bytes=100 * 1024 * 1024)


@jax.jit
def pallas_sequential_preLN__linear_kernel_hedgehog__geglu_ffn__prompt_kernel(
    A_x: jax.Array,
    A_wqkv: jax.Array,
    A_w_phi: jax.Array,
    A_wo: jax.Array,
    B_x: jax.Array,
    B_w_gate: jax.Array,
    B_w_up: jax.Array,
    B_w_down: jax.Array,
):
    T2, SB2, SBO, PS, NLOOP = 512, 256, 64, 2, 2
    x = A_x.reshape(S, D)
    wphi_t = jnp.transpose(A_w_phi, (1, 2, 0))
    anyspec = pl.BlockSpec(memory_space=pl.ANY)
    out = pl.pallas_call(
        functools.partial(_kernel, T2=T2, SB2=SB2, SBO=SBO, PS=PS, NLOOP=NLOOP),
        out_shape=jax.ShapeDtypeStruct((S, D), bf16),
        in_specs=[anyspec] * 7,
        out_specs=anyspec,
        scratch_shapes=[
            pltpu.VMEM((S // 2, D), u32),
            pltpu.VMEM((D // 2, 3 * D), u32),
            pltpu.VMEM((DH, DH, H), bf16),
            pltpu.VMEM((D // 2, D), u32),
            pltpu.VMEM((D // 2, F), u32),
            pltpu.VMEM((D // 2, F), u32),
            pltpu.VMEM((F // 2, D), u32),
            pltpu.VMEM((S, D), bf16),
            pltpu.VMEM((SB // 2, D), u32),
            pltpu.VMEM((3 * D // 2, D), u32),
            pltpu.VMEM((NG * 40, S), u32),
            pltpu.VMEM((NG * 40, 3 * SB), u32),
            pltpu.VMEM((NG * 24, 3 * SB), u32),
            pltpu.VMEM((NG * 48, 80), f32),
            pltpu.VMEM((NG * 24, 80), u32),
            pltpu.SemaphoreType.DMA((4,)),
            pltpu.SemaphoreType.DMA((8,)),
            pltpu.SemaphoreType.DMA((S // SBO,)),
        ],
        compiler_params=_compiler_params(),
    )(x, A_wqkv, wphi_t, A_wo, B_w_gate, B_w_up, B_w_down)
    return out.reshape(1, S, D)
```

```python
import functools
import jax
import jax.numpy as jnp
from jax import lax
import jax.experimental.pallas as pl
import jax.experimental.pallas.tpu as pltpu

S, D, H, DH, F = 2048, 640, 32, 20, 1536
NG = H // 2
GR = 2 * DH
DP = H * (DH - 1)
LOG2E = 1.4426950408889634
NT = (((1,), (1,)), ((), ()))
TN = (((0,), (0,)), ((), ()))
f32 = jnp.float32
bf16 = jnp.bfloat16
u32 = jnp.uint32
SB = 256
NSUB = S // SB
WROW = (0, DP, 2 * DP)
WLEN = (DP, DP, D)
TILES = [(64 * b, 64, 240 * (b // 2) + 112 * (b % 2), 128) for b in range(10)] + [(640, 48, 1200, 80)]


def _layernorm(x):
    m = jnp.mean(x, axis=-1, keepdims=True)
    xc = x - m
    v = jnp.mean(xc * xc, axis=-1, keepdims=True)
    return xc * lax.rsqrt(v + 1e-5)


def _recip(x):
    r = pl.reciprocal(x, approx=True)
    return r * (2.0 - x * r)


def _fold8(x, op):
    x = op(x, pltpu.roll(x, 2, 0))
    return op(x, pltpu.roll(x, 4, 0))


def _dual_softmax(p, split=False):
    T = p.shape[1]
    p3 = p.reshape(5, 8, T)
    mx = _fold8(jnp.max(p3, axis=0), jnp.maximum)
    mn = _fold8(jnp.min(p3, axis=0), jnp.minimum)
    ep = jnp.exp2(p3 - mx[None])
    en = jnp.exp2(mn[None] - p3)
    rp = _recip(_fold8(jnp.sum(ep, axis=0), jnp.add))
    rn = _recip(_fold8(jnp.sum(en, axis=0), jnp.add))
    ep = ep * rp[None]
    en = en * rn[None]
    if split:
        even = (lax.broadcasted_iota(jnp.int32, (5, 8, T), 1) & 1) == 0
        ep, en = (jnp.where(even, ep, pltpu.roll(en, 1, 1)), jnp.where(even, pltpu.roll(ep, 7, 1), en))
    phi = jnp.concatenate([ep, en], axis=0)
    return phi.reshape(2 * GR, T).astype(bf16)


def _group_logits(p):
    T = p.shape[1]
    pr = lax.broadcasted_iota(jnp.int32, (8, T), 0) >> 1
    out = []
    for q in range(p.shape[0] // 152):
        base = 152 * q
        xyz = [p[base + 8 * j:base + 8 * (j + 1)] for j in range(3)]
        last = [jnp.where(pr == j, 0.0, xyz[j]) for j in range(3)]
        last.append(jnp.where(pr == 0, xyz[0], jnp.where(pr == 1, xyz[1], jnp.where(pr == 2, xyz[2], 0.0))))
        for g in range(4):
            out.append(jnp.concatenate([last[g], p[base + 24 + 32 * g:base + 24 + 32 * (g + 1)]], axis=0))
    return out


def _pk(val):
    return pltpu.bitcast(val, u32)


def _upk(val):
    return pltpu.bitcast(val, bf16)


def _kernel(x_hbm, wqkv_hbm, wphi_hbm, wo_hbm, wg_hbm, wu_hbm, wd_hbm, out_hbm,
            x_v, wqkv_v, wphi_v, wo_v, wg_v, wu_v, wd_v, out_v,
            zs, xn_v, xn01, acc_s, wall, phiq, phik_s, vext_s, kvt, lmat, x_sem, w_sem, o_sem, *, T2, SB2, SBO, PS, NLOOP, KS, NU, AR):
    NB2 = S // T2

    xchunks = [(0, SB), (SB, SB), (2 * SB, 3 * SB), (5 * SB, 3 * SB)]
    wchunks = [(0, 1), (1, 2), (3, 2)]

    def x_copy(i):
        o, n = xchunks[i]
        return pltpu.make_async_copy(x_hbm.at[pl.ds(o, n)], x_v.at[pl.ds(o, n)], x_sem.at[i])

    def wqkv_copy(j):
        o, n = wchunks[j]
        return pltpu.make_async_copy(wqkv_hbm.at[pl.ds(o * 128, n * 128)], wqkv_v.at[pl.ds(o * 128, n * 128)],
                                     w_sem.at[j])

    def other(n):
        src, dst = ((wo_hbm, wo_v), (wg_hbm, wg_v), (wu_hbm, wu_v), (wd_hbm, wd_v), (wphi_hbm, wphi_v))[n]
        return pltpu.make_async_copy(src, dst, w_sem.at[3 + n])

    def out_copy(i):
        return pltpu.make_async_copy(out_v.at[pl.ds(i * SBO, SBO)], out_hbm.at[pl.ds(i * SBO, SBO)], o_sem.at[i])

    other(4).start()
    x_copy(0).start()
    x_copy(1).start()
    for j in range(3):
        wqkv_copy(j).start()
    x_copy(2).start()
    x_copy(3).start()
    zs[0] = 0

    hh = lax.broadcasted_iota(jnp.int32, (H, D), 0)
    cc = lax.broadcasted_iota(jnp.int32, (H, D), 1)
    inhead = (cc >= hh * DH) & (cc < hh * DH + DH)
    expand = jnp.where(inhead, 1.0, 0.0).astype(bf16)
    dcol = jnp.sum(jnp.where(inhead, cc - hh * DH, 0), axis=0, keepdims=True)

    def xyz_pattern(r):
        j = r >> 3
        p = (r >> 1) & 3
        par = r & 1
        f = jnp.where(p == j, 16 + j, 16 + p - jnp.where(p > j, 1, 0))
        hl = jnp.where(p == j, 6 + par, 2 * j + par)
        return f, hl

    r = lax.broadcasted_iota(jnp.int32, (56, DH), 0)
    j = lax.broadcasted_iota(jnp.int32, (56, DH), 1)
    frow = jnp.where(r < 32, r >> 1, xyz_pattern(r & 31)[0])
    a0 = jnp.where(frow == j, 1.0, jnp.where(j == DH - 1, -1.0, 0.0)).astype(bf16)
    other(4).wait()
    t0 = jnp.zeros((DH, D), f32)
    for d in range(DH):
        z = jnp.dot(wphi_v[d], expand, preferred_element_type=f32)
        t0 = jnp.where(dcol == d, z, t0)
    t0 = jnp.dot(a0, t0.astype(bf16), preferred_element_type=f32) * LOG2E

    blocks = []
    for q in range(4):
        for g in range(4):
            blocks.append((q, g))
            if g == 3 - q:
                blocks.append((q, 4))

    def tiles_of(q, kind):
        if kind == 4 or kind == 3 - q:
            return (q, q + 1)
        return (q,) if kind < 3 - q else (q + 1,)

    r = lax.broadcasted_iota(jnp.int32, (32, 128), 0)
    c = lax.broadcasted_iota(jnp.int32, (32, 128), 1)
    col_g = c - (r & 1) * DH
    col_x = (c - xyz_pattern(r)[1] * DH)[0:24]
    pts = []
    for t in range(5):
        mine = [b for b in blocks if t in tiles_of(*b)]
        parts = []
        for q, kind in mine:
            if kind == 4:
                rel, src = col_x + (128 * t - 160 * q), t0[32:56, 128 * t:128 * (t + 1)]
            else:
                rel, src = col_g + (128 * t - 160 * q - GR * kind), t0[0:32, 128 * t:128 * (t + 1)]
            parts.append(jnp.where((rel >= 0) & (rel < DH), src, 0.0))
        pts.append((mine, jnp.concatenate(parts, axis=0).astype(bf16)))

    def prep_chunk(c):
        o, n = wchunks[c]
        rows = slice(o * 128, (o + n) * 128)
        wall[WROW[2] // 2:(WROW[2] + D) // 2, rows] = _pk(wqkv_v[rows, 2 * D:3 * D].T)
        for j in (1, 0):
            res = {}
            for t, (mine, pt) in enumerate(pts):
                out = lax.dot_general(pt, wqkv_v[rows, j * D + 128 * t:j * D + 128 * (t + 1)], NT,
                                      preferred_element_type=f32)
                o2 = 0
                for b in mine:
                    nb = 24 if b[1] == 4 else 32
                    blk = out[o2:o2 + nb]
                    o2 += nb
                    res[b] = blk if b not in res else res[b] + blk
            parts = []
            for q in range(4):
                parts += [res[(q, k)] for k in (4, 0, 1, 2, 3)]
            wall[WROW[j] // 2:(WROW[j] + DP) // 2, rows] = _pk(jnp.concatenate(parts, axis=0).astype(bf16))

    def proj_part(j, k0, k1, nu=1):
        cols = slice(k0 * 128, k1 * 128)
        m = WLEN[j] // nu
        outs = []
        for u in range(nu):
            r0 = WROW[j] + u * m
            part = lax.dot_general(_upk(wall[r0 // 2:(r0 + m) // 2, cols]), _upk(xn01[:, cols]), NT,
                                   preferred_element_type=f32)
            if k0 > 0:
                part = part + acc_s[r0:r0 + m, :]
            if k1 < 5:
                acc_s[r0:r0 + m, :] = part
            outs.append(part)
        return jnp.concatenate(outs, axis=0)

    def ldx(off, n):
        return x_v[pl.ds(off, n), :].astype(f32)

    def ln1(off):
        return _layernorm(ldx(off, SB)).astype(bf16)

    def ln_next(off):
        vext_s[344:344 + AR // 2, 0:D] = _pk(_layernorm(ldx(off, AR)).astype(bf16))
        if AR < SB:
            xn_v[0:(SB - AR) // 2, :] = _pk(_layernorm(ldx(off + AR, SB - AR)).astype(bf16))

    def xn_next():
        parts = [vext_s[344:344 + AR // 2, 0:D]]
        if AR < SB:
            parts.append(xn_v[0:(SB - AR) // 2, :])
        return _upk(jnp.concatenate(parts, axis=0))

    def proj(j, xn):
        n = WLEN[j] // PS
        return jnp.concatenate(
            [lax.dot_general(_upk(wall[(WROW[j] + u * n) // 2:(WROW[j] + (u + 1) * n) // 2, :]), xn, NT,
                             preferred_element_type=f32) for u in range(PS)], axis=0)

    def sq(pq, off, g0=0):
        for g, lg in enumerate(_group_logits(pq)):
            phiq[40 * (g0 + g):40 * (g0 + g + 1), pl.ds(off, pq.shape[1])] = _pk(_dual_softmax(lg, (g0 + g) % 3 == 1))

    def sk(pk, slot, g0=0):
        for g, lg in enumerate(_group_logits(pk)):
            phik_s[40 * (g0 + g):40 * (g0 + g + 1), slot * SB:slot * SB + pk.shape[1]] = _pk(_dual_softmax(lg, (g0 + g) % 3 == 1))

    def sv(pv, slot, ts=range(6)):
        T = pv.shape[1]
        low = lax.broadcasted_iota(jnp.int32, (8, T), 0) < 4
        cols = slice(slot * SB, slot * SB + T)
        for t in [t for t in ts if t < 5]:
            mid = pv[120 * t + 56:120 * t + 64]
            blk = jnp.concatenate([pv[120 * t:120 * t + 56], jnp.where(low, mid, 1.0), jnp.where(low, 1.0, mid),
                                   pv[120 * t + 64:120 * t + 120]], axis=0)
            vext_s[64 * t:64 * (t + 1), cols] = _pk(blk.astype(bf16))
        if 5 in ts:
            vext_s[320:344, cols] = _pk(jnp.concatenate([pv[600:640], jnp.ones((8, T), f32)], axis=0).astype(bf16))

    def kv(slot, first=False, nslot=1, anchor=False):
        cols = slice(slot * SB, (slot + nslot) * SB)
        for r0, nr, f0, nf in TILES:
            rows = pl.ds(pl.multiple_of(zs[0], 8), nr // 2) if (anchor and r0 == 0) else pl.ds(r0 // 2, nr // 2)
            upd = lax.dot_general(_upk(vext_s[rows, cols]),
                                  _upk(phik_s[f0 // 2:(f0 + nf) // 2, cols]),
                                  NT, preferred_element_type=f32)
            if first:
                kvt[r0:r0 + nr, 0:nf] = upd
            else:
                kvt[r0:r0 + nr, 0:nf] += upd

    def pair(xna, off, noff, extra=None, extra_kv=None):
        pka = proj(1, xna)
        ex = [(proj(0, xn), o) for xn, o in (extra or [])]
        pqa = proj(0, xna)
        pva = proj(2, xna)
        sk(pka, 0)
        for pq, o in ex:
            sq(pq, o)
        sq(pqa, off)
        sv(pva, 0)
        if noff is not None:
            ln_next(noff)
        xnb = ln1(off + SB)
        pkb = proj(1, xnb)
        pqb = proj(0, xnb)
        pvb = proj(2, xnb)
        sk(pkb, 1)
        sq(pqb, off + SB)
        sv(pvb, 1, (0, 1))
        kv(0, anchor=True)
        sv(pvb, 1, (2, 3, 4, 5))
        kv(1)

    x_copy(0).wait()
    x_copy(1).wait()
    xn01[...] = _pk(_layernorm(ldx(0, 2 * SB)).astype(bf16))
    wqkv_copy(0).wait()
    prep_chunk(0)
    for j in (2, 1, 0):
        proj_part(j, 0, 1)
    wqkv_copy(1).wait()
    prep_chunk(1)
    proj_part(2, 1, 3)
    proj_part(1, 1, KS)
    proj_part(0, 1, KS)
    wqkv_copy(2).wait()
    x_copy(2).wait()
    for n in range(4):
        other(n).start()
    prep_chunk(2)
    pv01 = proj_part(2, 3, 5)
    xn2 = ln1(2 * SB)
    pk2 = proj(1, xn2)
    pk01 = proj_part(1, KS, 5, NU)
    pq2 = proj(0, xn2)
    pq01 = proj_part(0, KS, 5, NU)
    pv2 = proj(2, xn2)
    sv(pv01, 2)
    sk(pk2, 0)
    sk(pk01, 2)
    sq(pq2, 2 * SB)
    sq(pq01, 0)
    sv(pv2, 0)
    ln_next(4 * SB)
    xn3 = ln1(3 * SB)
    pk3 = proj(1, xn3)
    pq3 = proj(0, xn3)
    pv3 = proj(2, xn3)
    sk(pk3, 1)
    sq(pq3, 3 * SB)
    sv(pv3, 1, (0, 1))
    kv(2, first=True, nslot=2, anchor=True)
    sv(pv3, 1, (2, 3, 4, 5))
    kv(0)
    kv(1)
    nstraight = 1
    x_copy(3).wait()

    def phase1(i, carry):
        off = pl.multiple_of((2 + 2 * nstraight + i * 2) * SB, SB)
        noff = pl.multiple_of(jnp.minimum(4 + 2 * nstraight + i * 2, NSUB - 1) * SB, SB)
        pair(xn_next(), off, noff)
        return carry

    if NLOOP:
        lax.fori_loop(0, NLOOP, phase1, 0)

    r = lax.broadcasted_iota(jnp.int32, (64, 128), 0)
    c = lax.broadcasted_iota(jnp.int32, (64, 128), 1)

    def third(v):
        return jnp.where(v < DH, 0, jnp.where(v < GR, 1, 2))

    m_a = jnp.where(r < 60, third(r), jnp.minimum(r - 60, 2)) == jnp.where(c < 80, c & 1, jnp.where(c < 120, 2, 3))
    m_b = jnp.where(r < 4, jnp.minimum(r, 2), third(r - 4)) == jnp.where(c < 8, 3, jnp.where(c < 48, 0, 1 + (c & 1)))
    m_c = (jnp.where(r < GR, third(r), jnp.where(r < GR + 4, 0, 1)) == (c & 1))[0:48, 0:80]
    for b, (r0, nr, f0, nf) in enumerate(TILES):
        m = m_c if b == 10 else (m_a, m_b)[b % 2]
        lmat[r0 // 2:(r0 + nr) // 2, 0:nf] = _pk(jnp.where(m, kvt[r0:r0 + nr, 0:nf], 0.0).astype(bf16))

    for n in range(4):
        other(n).wait()

    def phase2(i, carry):
        off = pl.multiple_of(i * T2, T2)
        n = T2 // SB2
        low = lax.broadcasted_iota(jnp.int32, (8, SB2), 0) < 4
        ots = []
        for s in range(n):
            parts = []
            ogs = [jnp.dot(_upk(lmat[r0 // 2:(r0 + nr) // 2, 0:nf]),
                           _upk(phiq[f0 // 2:(f0 + nf) // 2, pl.ds(off + s * SB2, SB2)]),
                           preferred_element_type=f32) for r0, nr, f0, nf in TILES]
            for t in range(5):
                oa, ob = ogs[2 * t], ogs[2 * t + 1]
                rc = _recip(jnp.where(low, ob[0:8], oa[56:64]) + 1e-6)
                bc = [jnp.broadcast_to(rc[k:k + 1], (8, SB2)) for k in (4, 5, 6, 0, 1, 2)]
                parts += [oa[0:8] * bc[0], oa[8:16] * bc[0], oa[16:24] * jnp.where(low, bc[0], bc[1]),
                          oa[24:32] * bc[1], oa[32:40] * bc[1], oa[40:48] * bc[2], oa[48:56] * bc[2],
                          jnp.where(low, oa[56:64], ob[0:8]) * jnp.where(low, bc[2], bc[3]),
                          ob[8:16] * bc[3], ob[16:24] * bc[3], ob[24:32] * bc[4], ob[32:40] * bc[4],
                          ob[40:48] * jnp.where(low, bc[4], bc[5]), ob[48:56] * bc[5], ob[56:64] * bc[5]]
            og = ogs[10]
            rc = _recip(og[40:48] + 1e-6)
            rr = pltpu.roll(rc, 4, 0)
            r0_ = jnp.where(low, rc, rr)
            r1_ = jnp.where(low, rr, rc)
            parts += [og[0:8] * r0_, og[8:16] * r0_, og[16:24] * rc, og[24:32] * r1_, og[32:40] * r1_]
            ots.append(jnp.concatenate(parts, axis=0).astype(bf16))
        hs = []
        for s in range(n):
            attn = lax.dot_general(ots[s], wo_v[...], TN, preferred_element_type=f32)
            h = ldx(off + s * SB2, SB2) + attn
            hs.append((h, _layernorm(h).astype(bf16)))
        acts = []
        for s in range(n):
            hn = hs[s][1]
            gate = jnp.dot(hn, wg_v[...], preferred_element_type=f32)
            up = jnp.dot(hn, wu_v[...], preferred_element_type=f32)
            acts.append((jax.nn.gelu(gate, approximate=True) * up).astype(bf16))
        for s in range(n):
            for u in range(SB2 // SBO):
                y = hs[s][0][u * SBO:(u + 1) * SBO] + jnp.dot(acts[s][u * SBO:(u + 1) * SBO], wd_v[...],
                                                              preferred_element_type=f32)
                out_v[pl.ds(off + s * SB2 + u * SBO, SBO), :] = y.astype(bf16)
                out_copy(i * (T2 // SBO) + s * (SB2 // SBO) + u).start()
        return carry

    lax.fori_loop(0, NB2, phase2, 0)
    for i in range(S // SBO):
        out_copy(i).wait()


def _compiler_params():
    try:
        return pltpu.CompilerParams(vmem_limit_bytes=100 * 1024 * 1024, disable_bounds_checks=True,
                                    disable_semaphore_checks=True)
    except TypeError:
        return pltpu.CompilerParams(vmem_limit_bytes=100 * 1024 * 1024)


@jax.jit
def pallas_sequential_preLN__linear_kernel_hedgehog__geglu_ffn__prompt_kernel(
    A_x: jax.Array,
    A_wqkv: jax.Array,
    A_w_phi: jax.Array,
    A_wo: jax.Array,
    B_x: jax.Array,
    B_w_gate: jax.Array,
    B_w_up: jax.Array,
    B_w_down: jax.Array,
):
    T2 = 512
    SB2 = 256
    SBO = 64
    PS = 2
    NLOOP = 2
    KS = 2
    NU = 2
    AR = 128
    x = A_x.reshape(S, D)
    wphi_t = jnp.transpose(A_w_phi, (1, 2, 0))
    anyspec = pl.BlockSpec(memory_space=pl.ANY)
    out = pl.pallas_call(
        functools.partial(_kernel, T2=T2, SB2=SB2, SBO=SBO, PS=PS, NLOOP=NLOOP, KS=KS, NU=NU, AR=AR),
        out_shape=jax.ShapeDtypeStruct((S, D), bf16),
        in_specs=[anyspec] * 7,
        out_specs=anyspec,
        scratch_shapes=[
            pltpu.VMEM((S, D), bf16),
            pltpu.VMEM((D, 3 * D), bf16),
            pltpu.VMEM((DH, DH, H), bf16),
            pltpu.VMEM((D, D), bf16),
            pltpu.VMEM((D, F), bf16),
            pltpu.VMEM((D, F), bf16),
            pltpu.VMEM((F, D), bf16),
            pltpu.VMEM((S, D), bf16),
            pltpu.SMEM((1,), jnp.int32),
            pltpu.VMEM((SB // 2, D), u32),
            pltpu.VMEM((SB, D), u32),
            pltpu.VMEM((2 * DP + D, 2 * SB), f32),
            pltpu.VMEM(((2 * DP + D) // 2, D), u32),
            pltpu.VMEM((NG * 40, S), u32),
            pltpu.VMEM((NG * 40, 4 * SB), u32),
            pltpu.VMEM((344 + SB // 2, 4 * SB), u32),
            pltpu.VMEM((688, 128), f32),
            pltpu.VMEM((344, 128), u32),
            pltpu.SemaphoreType.DMA((4,)),
            pltpu.SemaphoreType.DMA((8,)),
            pltpu.SemaphoreType.DMA((S // SBO,)),
        ],
        compiler_params=_compiler_params(),
    )(x, A_wqkv, wphi_t, A_wo, B_w_gate, B_w_up, B_w_down)
    return out.reshape(1, S, D)
```

```python
import functools
import jax
import jax.numpy as jnp
from jax import lax
import jax.experimental.pallas as pl
import jax.experimental.pallas.tpu as pltpu

S, D, H, DH, F = 2048, 640, 32, 20, 1536
NG = H // 2
GR = 2 * DH
DP = H * (DH - 1)
LOG2E = 1.4426950408889634
NT = (((1,), (1,)), ((), ()))
TN = (((0,), (0,)), ((), ()))
f32 = jnp.float32
bf16 = jnp.bfloat16
u32 = jnp.uint32
SB = 256
NSUB = S // SB
WROW = (0, DP, 2 * DP)
WLEN = (DP, DP, D)
TILES = [(64 * b, 64, 240 * (b // 2) + 112 * (b % 2), 128) for b in range(10)] + [(640, 48, 1200, 80)]


def _layernorm(x, alt=False):
    m = jnp.mean(x, axis=-1, keepdims=True)
    xc = x - m
    v = jnp.mean(xc * xc, axis=-1, keepdims=True)
    r = lax.rsqrt(v + 1e-5)
    if alt:
        return x * r - m * r
    return xc * r


def _recip(x):
    r = pl.reciprocal(x, approx=True)
    return r * (2.0 - x * r)


def _fold8(x, op):
    x = op(x, pltpu.roll(x, 2, 0))
    return op(x, pltpu.roll(x, 4, 0))


def _dual_softmax(p, split=False):
    T = p.shape[1]
    p3 = p.reshape(5, 8, T)
    mx = _fold8(jnp.max(p3, axis=0), jnp.maximum)
    mn = _fold8(jnp.min(p3, axis=0), jnp.minimum)
    ep = jnp.exp2(p3 - mx[None])
    en = jnp.exp2(mn[None] - p3)
    rp = _recip(_fold8(jnp.sum(ep, axis=0), jnp.add))
    rn = _recip(_fold8(jnp.sum(en, axis=0), jnp.add))
    ep = ep * rp[None]
    en = en * rn[None]
    if split:
        even = (lax.broadcasted_iota(jnp.int32, (5, 8, T), 1) & 1) == 0
        ep, en = (jnp.where(even, ep, pltpu.roll(en, 1, 1)), jnp.where(even, pltpu.roll(ep, 7, 1), en))
    phi = jnp.concatenate([ep, en], axis=0)
    return phi.reshape(2 * GR, T).astype(bf16)


def _group_logits(p):
    T = p.shape[1]
    pr = lax.broadcasted_iota(jnp.int32, (8, T), 0) >> 1
    out = []
    for q in range(p.shape[0] // 152):
        base = 152 * q
        xyz = [p[base + 8 * j:base + 8 * (j + 1)] for j in range(3)]
        last = [jnp.where(pr == j, 0.0, xyz[j]) for j in range(3)]
        last.append(jnp.where(pr == 0, xyz[0], jnp.where(pr == 1, xyz[1], jnp.where(pr == 2, xyz[2], 0.0))))
        for g in range(4):
            out.append(jnp.concatenate([last[g], p[base + 24 + 32 * g:base + 24 + 32 * (g + 1)]], axis=0))
    return out


def _pk(val):
    return pltpu.bitcast(val, u32)


def _upk(val):
    return pltpu.bitcast(val, bf16)


def _kernel(x_hbm, wqkv_hbm, wphi_hbm, wo_hbm, wg_hbm, wu_hbm, wd_hbm, out_hbm,
            x_v, wqkv_v, wphi_v, wo_v, wg_v, wu_v, wd_v, out_v,
            zs, xn_v, xn01, acc_s, wall, phiq, phik_s, vext_s, kvt, lmat, d_s, x_sem, w_sem, o_sem, *, T2, SB2, SBO, PS, NLOOP, KS, NU, AR, NCH, NA, KD, ALT, ORD):
    NB2 = S // T2

    xchunks = [(0, SB), (SB, SB), (2 * SB, 3 * SB), (5 * SB, 3 * SB)]
    wchunks = [(0, 1), (1, 2), (3, 2)]

    def x_copy(i):
        o, n = xchunks[i]
        return pltpu.make_async_copy(x_hbm.at[pl.ds(o, n)], x_v.at[pl.ds(o, n)], x_sem.at[i])

    def wqkv_copy(j):
        o, n = wchunks[j]
        return pltpu.make_async_copy(wqkv_hbm.at[pl.ds(o * 128, n * 128)], wqkv_v.at[pl.ds(o * 128, n * 128)],
                                     w_sem.at[j])

    def other(n):
        src, dst = ((wo_hbm, wo_v), (wg_hbm, wg_v), (wu_hbm, wu_v), (wd_hbm, wd_v), (wphi_hbm, wphi_v))[n]
        return pltpu.make_async_copy(src, dst, w_sem.at[3 + n])

    def out_copy(i):
        return pltpu.make_async_copy(out_v.at[pl.ds(i * SBO, SBO)], out_hbm.at[pl.ds(i * SBO, SBO)], o_sem.at[i])

    other(4).start()
    x_copy(0).start()
    x_copy(1).start()
    for j in range(3):
        wqkv_copy(j).start()
    x_copy(2).start()
    x_copy(3).start()
    zs[0] = 0

    hh = lax.broadcasted_iota(jnp.int32, (H, D), 0)
    cc = lax.broadcasted_iota(jnp.int32, (H, D), 1)
    inhead = (cc >= hh * DH) & (cc < hh * DH + DH)
    expand = jnp.where(inhead, 1.0, 0.0).astype(bf16)
    dcol = jnp.sum(jnp.where(inhead, cc - hh * DH, 0), axis=0, keepdims=True)

    def xyz_pattern(r):
        j = r >> 3
        p = (r >> 1) & 3
        par = r & 1
        f = jnp.where(p == j, 16 + j, 16 + p - jnp.where(p > j, 1, 0))
        hl = jnp.where(p == j, 6 + par, 2 * j + par)
        return f, hl

    r = lax.broadcasted_iota(jnp.int32, (56, DH), 0)
    j = lax.broadcasted_iota(jnp.int32, (56, DH), 1)
    frow = jnp.where(r < 32, r >> 1, xyz_pattern(r & 31)[0])
    a0 = jnp.where(frow == j, 1.0, jnp.where(j == DH - 1, -1.0, 0.0)).astype(bf16)
    other(4).wait()
    t0 = jnp.zeros((DH, D), f32)
    for d in range(DH):
        z = jnp.dot(wphi_v[d], expand, preferred_element_type=f32)
        t0 = jnp.where(dcol == d, z, t0)
    t0 = jnp.dot(a0, t0.astype(bf16), preferred_element_type=f32) * LOG2E

    blocks = []
    for q in range(4):
        for g in range(4):
            blocks.append((q, g))
            if g == 3 - q:
                blocks.append((q, 4))

    def tiles_of(q, kind):
        if kind == 4 or kind == 3 - q:
            return (q, q + 1)
        return (q,) if kind < 3 - q else (q + 1,)

    r = lax.broadcasted_iota(jnp.int32, (32, 128), 0)
    c = lax.broadcasted_iota(jnp.int32, (32, 128), 1)
    col_g = c - (r & 1) * DH
    col_x = (c - xyz_pattern(r)[1] * DH)[0:24]
    pts = []
    for t in range(5):
        mine = [b for b in blocks if t in tiles_of(*b)]
        parts = []
        for q, kind in mine:
            if kind == 4:
                rel, src = col_x + (128 * t - 160 * q), t0[32:56, 128 * t:128 * (t + 1)]
            else:
                rel, src = col_g + (128 * t - 160 * q - GR * kind), t0[0:32, 128 * t:128 * (t + 1)]
            parts.append(jnp.where((rel >= 0) & (rel < DH), src, 0.0))
        pts.append((mine, jnp.concatenate(parts, axis=0).astype(bf16)))

    def prep_chunk(c):
        o, n = wchunks[c]
        rows = slice(o * 128, (o + n) * 128)
        wall[WROW[2] // 2:(WROW[2] + D) // 2, rows] = _pk(wqkv_v[rows, 2 * D:3 * D].T)
        for j in (1, 0):
            res = {}
            for t, (mine, pt) in enumerate(pts):
                out = lax.dot_general(pt, wqkv_v[rows, j * D + 128 * t:j * D + 128 * (t + 1)], NT,
                                      preferred_element_type=f32)
                o2 = 0
                for b in mine:
                    nb = 24 if b[1] == 4 else 32
                    blk = out[o2:o2 + nb]
                    o2 += nb
                    res[b] = blk if b not in res else res[b] + blk
            parts = []
            for q in range(4):
                parts += [res[(q, k)] for k in (4, 0, 1, 2, 3)]
            wall[WROW[j] // 2:(WROW[j] + DP) // 2, rows] = _pk(jnp.concatenate(parts, axis=0).astype(bf16))

    def proj_part(j, k0, k1, nu=1):
        cols = slice(k0 * 128, k1 * 128)
        m = WLEN[j] // nu
        outs = []
        for u in range(nu):
            r0 = WROW[j] + u * m
            part = lax.dot_general(_upk(wall[r0 // 2:(r0 + m) // 2, cols]), _upk(xn01[:, cols]), NT,
                                   preferred_element_type=f32)
            if k0 > 0:
                part = part + acc_s[r0:r0 + m, :]
            if k1 < 5:
                acc_s[r0:r0 + m, :] = part
            outs.append(part)
        return jnp.concatenate(outs, axis=0)

    def ldx(off, n):
        return x_v[pl.ds(off, n), :].astype(f32)

    def ln1(off):
        return _layernorm(ldx(off, SB)).astype(bf16)

    def ln_next(off):
        vext_s[344:344 + AR // 2, 0:D] = _pk(_layernorm(ldx(off, AR)).astype(bf16))
        if AR < SB:
            xn_v[0:(SB - AR) // 2, :] = _pk(_layernorm(ldx(off + AR, SB - AR)).astype(bf16))

    def xn_next():
        parts = [vext_s[344:344 + AR // 2, 0:D]]
        if AR < SB:
            parts.append(xn_v[0:(SB - AR) // 2, :])
        return _upk(jnp.concatenate(parts, axis=0))

    def proj(j, xn):
        n = WLEN[j] // PS
        return jnp.concatenate(
            [lax.dot_general(_upk(wall[(WROW[j] + u * n) // 2:(WROW[j] + (u + 1) * n) // 2, :]), xn, NT,
                             preferred_element_type=f32) for u in range(PS)], axis=0)

    def sq(pq, off, g0=0):
        for g, lg in enumerate(_group_logits(pq)):
            phiq[40 * (g0 + g):40 * (g0 + g + 1), pl.ds(off, pq.shape[1])] = _pk(_dual_softmax(lg, (g0 + g) % 3 == 1))

    def sk(pk, slot, g0=0):
        for g, lg in enumerate(_group_logits(pk)):
            phik_s[40 * (g0 + g):40 * (g0 + g + 1), slot * SB:slot * SB + pk.shape[1]] = _pk(_dual_softmax(lg, (g0 + g) % 3 == 1))

    def sv(pv, slot, ts=range(6)):
        T = pv.shape[1]
        low = lax.broadcasted_iota(jnp.int32, (8, T), 0) < 4
        cols = slice(slot * SB, slot * SB + T)
        for t in [t for t in ts if t < 5]:
            mid = pv[120 * t + 56:120 * t + 64]
            blk = jnp.concatenate([pv[120 * t:120 * t + 56], jnp.where(low, mid, 1.0), jnp.where(low, 1.0, mid),
                                   pv[120 * t + 64:120 * t + 120]], axis=0)
            vext_s[64 * t:64 * (t + 1), cols] = _pk(blk.astype(bf16))
        if 5 in ts:
            vext_s[320:344, cols] = _pk(jnp.concatenate([pv[600:640], jnp.ones((8, T), f32)], axis=0).astype(bf16))

    def kv(slot, first=False, nslot=1, anchor=False):
        cols = slice(slot * SB, (slot + nslot) * SB)
        for r0, nr, f0, nf in TILES:
            rows = pl.ds(pl.multiple_of(zs[0], 8), nr // 2) if (anchor and r0 == 0) else pl.ds(r0 // 2, nr // 2)
            upd = lax.dot_general(_upk(vext_s[rows, cols]),
                                  _upk(phik_s[f0 // 2:(f0 + nf) // 2, cols]),
                                  NT, preferred_element_type=f32)
            if first:
                kvt[r0:r0 + nr, 0:nf] = upd
            else:
                kvt[r0:r0 + nr, 0:nf] += upd

    def pair(xna, off, noff, extra=None, extra_kv=None):
        pka = proj(1, xna)
        ex = [(proj(0, xn), o) for xn, o in (extra or [])]
        pqa = proj(0, xna)
        pva = proj(2, xna)
        sk(pka, 0)
        for pq, o in ex:
            sq(pq, o)
        sq(pqa, off)
        sv(pva, 0)
        if noff is not None:
            ln_next(noff)
        xnb = ln1(off + SB)
        pkb = proj(1, xnb)
        pqb = proj(0, xnb)
        pvb = proj(2, xnb)
        sk(pkb, 1)
        sq(pqb, off + SB)
        sv(pvb, 1, (0, 1))
        kv(0, anchor=True)
        sv(pvb, 1, (2, 3, 4, 5))
        kv(1)

    x_copy(0).wait()
    x_copy(1).wait()
    xn01[...] = _pk(_layernorm(ldx(0, 2 * SB)).astype(bf16))
    wqkv_copy(0).wait()
    prep_chunk(0)
    for j in (2, 1, 0):
        proj_part(j, 0, 1)
    wqkv_copy(1).wait()
    prep_chunk(1)
    proj_part(2, 1, 3)
    proj_part(1, 1, KS)
    proj_part(0, 1, KS)
    wqkv_copy(2).wait()
    x_copy(2).wait()
    for n in range(4):
        other(n).start()
    prep_chunk(2)
    pv01 = proj_part(2, 3, 5)
    xn2 = ln1(2 * SB)
    pk2 = proj(1, xn2)
    pk01 = proj_part(1, KS, 5, NU)
    pq2 = proj(0, xn2)
    pq01 = proj_part(0, KS, 5, NU)
    pv2 = proj(2, xn2)
    sv(pv01, 2)
    sk(pk2, 0)
    sk(pk01, 2)
    sq(pq2, 2 * SB)
    sq(pq01, 0)
    sv(pv2, 0)
    ln_next(4 * SB)
    xn3 = ln1(3 * SB)
    pk3 = proj(1, xn3)
    pq3 = proj(0, xn3)
    pv3 = proj(2, xn3)
    sk(pk3, 1)
    sq(pq3, 3 * SB)
    sv(pv3, 1, (0, 1))
    kv(2, first=True, nslot=2, anchor=True)
    sv(pv3, 1, (2, 3, 4, 5))
    kv(0)
    kv(1)
    nstraight = 1
    x_copy(3).wait()

    def phase1(i, carry):
        off = pl.multiple_of((2 + 2 * nstraight + i * 2) * SB, SB)
        noff = pl.multiple_of(jnp.minimum(4 + 2 * nstraight + i * 2, NSUB - 1) * SB, SB)
        pair(xn_next(), off, noff)
        return carry

    if NLOOP:
        lax.fori_loop(0, NLOOP, phase1, 0)

    r = lax.broadcasted_iota(jnp.int32, (64, 128), 0)
    c = lax.broadcasted_iota(jnp.int32, (64, 128), 1)

    def third(v):
        return jnp.where(v < DH, 0, jnp.where(v < GR, 1, 2))

    m_a = jnp.where(r < 60, third(r), jnp.minimum(r - 60, 2)) == jnp.where(c < 80, c & 1, jnp.where(c < 120, 2, 3))
    m_b = jnp.where(r < 4, jnp.minimum(r, 2), third(r - 4)) == jnp.where(c < 8, 3, jnp.where(c < 48, 0, 1 + (c & 1)))
    m_c = (jnp.where(r < GR, third(r), jnp.where(r < GR + 4, 0, 1)) == (c & 1))[0:48, 0:80]
    for b, (r0, nr, f0, nf) in enumerate(TILES):
        m = m_c if b == 10 else (m_a, m_b)[b % 2]
        lmat[r0 // 2:(r0 + nr) // 2, 0:nf] = _pk(jnp.where(m, kvt[r0:r0 + nr, 0:nf], 0.0).astype(bf16))

    for n in range(4):
        other(n).wait()

    def phase2(i, carry):
        off = pl.multiple_of(i * T2, T2)
        n = T2 // SB2
        low = lax.broadcasted_iota(jnp.int32, (8, SB2), 0) < 4
        ots = []
        for s in range(n):
            parts = []
            ogs = [jnp.dot(_upk(lmat[r0 // 2:(r0 + nr) // 2, 0:nf]),
                           _upk(phiq[f0 // 2:(f0 + nf) // 2, pl.ds(off + s * SB2, SB2)]),
                           preferred_element_type=f32) for r0, nr, f0, nf in TILES]
            for t in range(5):
                oa, ob = ogs[2 * t], ogs[2 * t + 1]
                rc = _recip(jnp.where(low, ob[0:8], oa[56:64]) + 1e-6)
                bc = [jnp.broadcast_to(rc[k:k + 1], (8, SB2)) for k in (4, 5, 6, 0, 1, 2)]
                parts += [oa[0:8] * bc[0], oa[8:16] * bc[0], oa[16:24] * jnp.where(low, bc[0], bc[1]),
                          oa[24:32] * bc[1], oa[32:40] * bc[1], oa[40:48] * bc[2], oa[48:56] * bc[2],
                          jnp.where(low, oa[56:64], ob[0:8]) * jnp.where(low, bc[2], bc[3]),
                          ob[8:16] * bc[3], ob[16:24] * bc[3], ob[24:32] * bc[4], ob[32:40] * bc[4],
                          ob[40:48] * jnp.where(low, bc[4], bc[5]), ob[48:56] * bc[5], ob[56:64] * bc[5]]
            og = ogs[10]
            rc = _recip(og[40:48] + 1e-6)
            rr = pltpu.roll(rc, 4, 0)
            r0_ = jnp.where(low, rc, rr)
            r1_ = jnp.where(low, rr, rc)
            parts += [og[0:8] * r0_, og[8:16] * r0_, og[16:24] * rc, og[24:32] * r1_, og[32:40] * r1_]
            ots.append(jnp.concatenate(parts, axis=0).astype(bf16))
        hs = []
        for s in range(n):
            attn = lax.dot_general(ots[s], wo_v[...], TN, preferred_element_type=f32)
            h = ldx(off + s * SB2, SB2) + attn
            hs.append((h, _layernorm(h, ALT)))

        def mm(x, y):
            return jnp.dot(x, y, preferred_element_type=f32)

        def cat(axis, *vs):
            return jnp.concatenate(vs, axis=axis)

        ha, hb = hs[0][1], hs[1][1]
        a11, a12, a21, a22 = ha[:, 0:256], ha[:, 256:512], hb[:, 0:256], hb[:, 256:512]
        ra, rb = ha[:, 512:D], hb[:, 512:D]
        s1, s2r, s3, s4, s5r, s6r, s7r = [v.astype(bf16) for v in (
            a11 + a22, cat(1, a21 + a22, rb), a11, a22, cat(1, a11 + a12, ra), cat(1, a21 - a11, rb),
            cat(1, a12 - a22, ra))]
        HF = F // 2
        CW = HF // NCH

        def wcols(r0, r1, c0):
            return cat(1, wg_v[r0:r1, c0:c0 + CW], wu_v[r0:r1, c0:c0 + CW])

        def wcols32(r0, r1, c0):
            return cat(1, wg_v[r0:r1, c0:c0 + CW].astype(f32), wu_v[r0:r1, c0:c0 + CW].astype(f32))

        def glu(c):
            return jax.nn.gelu(c[:, 0:CW], approximate=True) * c[:, CW:2 * CW]

        m5s = [mm(s5r, wcols(256, D, HF + c * CW)) for c in range(NA)]
        for c in range(NCH):
            c1, c2 = c * CW, HF + c * CW
            f11, f12, f21, f22 = wcols32(0, 256, c1), wcols32(0, 256, c2), wcols32(256, 512, c1), wcols32(256, 512, c2)
            r12 = wcols32(512, D, c1) + wcols32(512, D, c2)
            m5 = m5s[c] if c < NA else mm(s5r, wcols(256, D, c2))
            m2 = mm(s2r, cat(0, wcols(0, 256, c1), wcols(512, D, c1)))
            m1 = mm(s1, (f11 + f22).astype(bf16))
            p22 = m1 - m2
            p11 = m1 - m5
            m3 = mm(s3, (f12 - f22).astype(bf16))
            c12 = m3 + m5
            p22 = p22 + m3
            if ORD == 0:
                m4 = mm(s4, (f21 - f11).astype(bf16))
                c21 = m2 + m4
                p11 = p11 + m4
                c11 = p11 + mm(s7r, cat(0, f21 + f22, r12).astype(bf16))
                c22 = p22 + mm(s6r, cat(0, f11 + f12, r12).astype(bf16))
            else:
                c22 = p22 + mm(s6r, cat(0, f11 + f12, r12).astype(bf16))
                m4 = mm(s4, (f21 - f11).astype(bf16))
                c21 = m2 + m4
                p11 = p11 + m4
                c11 = p11 + mm(s7r, cat(0, f21 + f22, r12).astype(bf16))
            q11, q12, q21, q22 = glu(c11), glu(c12), glu(c21), glu(c22)
            for k, v in enumerate((q11 + q22, q21 + q22, q11, q22, q11 + q12, q21 - q11, q12 - q22, q12, q21)):
                d_s[:, k * HF + c * CW:k * HF + (c + 1) * CW] = _pk(v.astype(bf16))

        def dn_rhs(k0, k1):
            f11, f12 = wd_v[k0:k1, 0:256].astype(f32), wd_v[k0:k1, 256:512].astype(f32)
            f21, f22 = wd_v[HF + k0:HF + k1, 0:256].astype(f32), wd_v[HF + k0:HF + k1, 256:512].astype(f32)
            w4 = cat(0, wd_v[k0:k1, 512:D], wd_v[HF + k0:HF + k1, 512:D])
            return [(f11 + f22).astype(bf16), wd_v[k0:k1, 0:256], (f12 - f22).astype(bf16), (f21 - f11).astype(bf16),
                    wd_v[HF + k0:HF + k1, 256:512], (f11 + f12).astype(bf16), (f21 + f22).astype(bf16), w4, w4]

        def dn(k, r0, r1, k0, k1, t):
            rows = slice(r0 // 2, r1 // 2)
            if k < 7:
                return mm(_upk(d_s[rows, k * HF + k0:k * HF + k1]), t[k])
            lo, hi = ((2, 7), (8, 3))[k - 7]
            return mm(_upk(cat(1, d_s[rows, lo * HF + k0:lo * HF + k1], d_s[rows, hi * HF + k0:hi * HF + k1])), t[k])

        first = {}
        if KD:
            t = dn_rhs(0, KD)
            for k in (7, 8, 4, 1, 2, 3, 0, 6, 5):
                first[k] = dn(k, 0, SB2, 0, KD, t)
        t = dn_rhs(KD, HF)
        for u in range(SB2 // SBO):
            rows = slice(u * SBO, (u + 1) * SBO)

            def fin(k):
                v = dn(k, u * SBO, (u + 1) * SBO, KD, HF, t)
                return v + first[k][rows] if KD else v

            ya4 = fin(7)
            m5, m3, m1, m4, m7 = [fin(k) for k in (4, 2, 0, 3, 6)]
            ya = cat(1, m1 + m4 - m5 + m7, m3 + m5, ya4) + hs[0][0][rows]
            out_v[pl.ds(off + u * SBO, SBO), :] = ya.astype(bf16)
            out_copy(i * (T2 // SBO) + u).start()
            yb4 = fin(8)
            m2, m6 = fin(1), fin(5)
            yb = cat(1, m2 + m4, m1 - m2 + m3 + m6, yb4) + hs[1][0][rows]
            out_v[pl.ds(off + SB2 + u * SBO, SBO), :] = yb.astype(bf16)
            out_copy(i * (T2 // SBO) + SB2 // SBO + u).start()
        return carry

    lax.fori_loop(0, NB2, phase2, 0)
    for i in range(S // SBO):
        out_copy(i).wait()


def _compiler_params():
    try:
        return pltpu.CompilerParams(vmem_limit_bytes=100 * 1024 * 1024, disable_bounds_checks=True,
                                    disable_semaphore_checks=True)
    except TypeError:
        return pltpu.CompilerParams(vmem_limit_bytes=100 * 1024 * 1024)


@jax.jit
def pallas_sequential_preLN__linear_kernel_hedgehog__geglu_ffn__prompt_kernel(
    A_x: jax.Array,
    A_wqkv: jax.Array,
    A_w_phi: jax.Array,
    A_wo: jax.Array,
    B_x: jax.Array,
    B_w_gate: jax.Array,
    B_w_up: jax.Array,
    B_w_down: jax.Array,
):
    T2 = 512
    SB2 = 256
    SBO = 64
    PS = 2
    NLOOP = 2
    KS = 2
    NU = 2
    AR = 128
    NCH = 3
    NA = 2
    KD = 512
    ALT = 0
    ORD = 0
    x = A_x.reshape(S, D)
    wphi_t = jnp.transpose(A_w_phi, (1, 2, 0))
    anyspec = pl.BlockSpec(memory_space=pl.ANY)
    out = pl.pallas_call(
        functools.partial(_kernel, T2=T2, SB2=SB2, SBO=SBO, PS=PS, NLOOP=NLOOP, KS=KS, NU=NU, AR=AR, NCH=NCH, NA=NA, KD=KD, ALT=ALT, ORD=ORD),
        out_shape=jax.ShapeDtypeStruct((S, D), bf16),
        in_specs=[anyspec] * 7,
        out_specs=anyspec,
        scratch_shapes=[
            pltpu.VMEM((S, D), bf16),
            pltpu.VMEM((D, 3 * D), bf16),
            pltpu.VMEM((DH, DH, H), bf16),
            pltpu.VMEM((D, D), bf16),
            pltpu.VMEM((D, F), bf16),
            pltpu.VMEM((D, F), bf16),
            pltpu.VMEM((F, D), bf16),
            pltpu.VMEM((S, D), bf16),
            pltpu.SMEM((1,), jnp.int32),
            pltpu.VMEM((SB // 2, D), u32),
            pltpu.VMEM((SB, D), u32),
            pltpu.VMEM((2 * DP + D, 2 * SB), f32),
            pltpu.VMEM(((2 * DP + D) // 2, D), u32),
            pltpu.VMEM((NG * 40, S), u32),
            pltpu.VMEM((NG * 40, 4 * SB), u32),
            pltpu.VMEM((344 + SB // 2, 4 * SB), u32),
            pltpu.VMEM((688, 128), f32),
            pltpu.VMEM((344, 128), u32),
            pltpu.VMEM((SB2 // 2, 9 * F // 2), u32),
            pltpu.SemaphoreType.DMA((4,)),
            pltpu.SemaphoreType.DMA((8,)),
            pltpu.SemaphoreType.DMA((S // SBO,)),
        ],
        compiler_params=_compiler_params(),
    )(x, A_wqkv, wphi_t, A_wo, B_w_gate, B_w_up, B_w_down)
    return out.reshape(1, S, D)
```

```python
import jax
import jax.numpy as jnp
from jax import lax
import jax.experimental.pallas as pl
import jax.experimental.pallas.tpu as pltpu

S, D, H, DH, F = 2048, 640, 32, 20, 1536
NG = H // 2
GR = 2 * DH
DP = H * (DH - 1)
HF = F // 2
LOG2E = 1.4426950408889634
NT = (((1,), (1,)), ((), ()))
TN = (((0,), (0,)), ((), ()))
f32 = jnp.float32
bf16 = jnp.bfloat16
u32 = jnp.uint32
SB = 256
NSUB = S // SB
WROW = (0, DP, 2 * DP)
WLEN = (DP, DP, D)
HROW = (0, DP // 2, DP)
XROW = (2 * DP + D) // 2
TILES = [(64 * b, 64, 240 * (b // 2) + 112 * (b % 2), 128) for b in range(10)] + [(640, 48, 1200, 80)]
XCHUNKS = [(0, SB), (SB, SB), (2 * SB, SB), (3 * SB, 5 * SB)]
WCHUNKS = [(0, 1), (1, 2), (3, 2)]
AR = 128
NCH = 3
CW = HF // NCH
NA = 2
KD = 512
CH = (128, 64, 64)


def _layernorm(x):
    m = jnp.mean(x, axis=-1, keepdims=True)
    xc = x - m
    v = jnp.mean(xc * xc, axis=-1, keepdims=True)
    return xc * lax.rsqrt(v + 1e-5)


def _recip(x):
    r = pl.reciprocal(x, approx=True)
    return r * (2.0 - x * r)


def _fold8(x, op):
    x = op(x, pltpu.roll(x, 2, 0))
    return op(x, pltpu.roll(x, 4, 0))


def _dual_softmax(p, split):
    T = p.shape[1]
    p3 = p.reshape(5, 8, T)
    mx = _fold8(jnp.max(p3, axis=0), jnp.maximum)
    mn = _fold8(jnp.min(p3, axis=0), jnp.minimum)
    ep = jnp.exp2(p3 - mx[None])
    en = jnp.exp2(mn[None] - p3)
    ep = ep * _recip(_fold8(jnp.sum(ep, axis=0), jnp.add))[None]
    en = en * _recip(_fold8(jnp.sum(en, axis=0), jnp.add))[None]
    if split:
        even = (lax.broadcasted_iota(jnp.int32, (5, 8, T), 1) & 1) == 0
        ep, en = (jnp.where(even, ep, pltpu.roll(en, 1, 1)), jnp.where(even, pltpu.roll(ep, 7, 1), en))
    return jnp.concatenate([ep, en], axis=0).reshape(2 * GR, T).astype(bf16)


def _group_logits(p):
    T = p.shape[1]
    pr = lax.broadcasted_iota(jnp.int32, (8, T), 0) >> 1
    out = []
    for q in range(p.shape[0] // 152):
        base = 152 * q
        xyz = [p[base + 8 * j:base + 8 * (j + 1)] for j in range(3)]
        last = [jnp.where(pr == j, 0.0, xyz[j]) for j in range(3)]
        last.append(jnp.where(pr == 0, xyz[0], jnp.where(pr == 1, xyz[1], jnp.where(pr == 2, xyz[2], 0.0))))
        for g in range(4):
            out.append(jnp.concatenate([last[g], p[base + 24 + 32 * g:base + 24 + 32 * (g + 1)]], axis=0))
    return out


def _pk(val):
    return pltpu.bitcast(val, u32)


def _upk(val):
    return pltpu.bitcast(val, bf16)


def _cat(axis, *vs):
    return jnp.concatenate(vs, axis=axis)


def _mm(x, y):
    return jnp.dot(x, y, preferred_element_type=f32)


def _mm_nt(x, y):
    return lax.dot_general(x, y, NT, preferred_element_type=f32)


def _kernel(x_hbm, wqkv_hbm, wphi_hbm, wo_hbm, wg_hbm, wu_hbm, wd_hbm, out_hbm,
            x_v, wqkv_v, wphi_v, wo_v, wg_v, wu_v, wd_v, out_v,
            zs, xn_v, xn01, acc_s, wall, wcmb, phiq, phik_s, vext_s, kvt, lmat, d_s, x_sem, w_sem, o_sem):

    def x_copy(i):
        o, n = XCHUNKS[i]
        return pltpu.make_async_copy(x_hbm.at[pl.ds(o, n)], x_v.at[pl.ds(o, n)], x_sem.at[i])

    def wqkv_copy(j):
        o, n = WCHUNKS[j]
        return pltpu.make_async_copy(wqkv_hbm.at[pl.ds(o * 128, n * 128)], wqkv_v.at[pl.ds(o * 128, n * 128)],
                                     w_sem.at[j])

    def other(n):
        src, dst = ((wo_hbm, wo_v), (wg_hbm, wg_v), (wu_hbm, wu_v), (wd_hbm, wd_v), (wphi_hbm, wphi_v))[n]
        return pltpu.make_async_copy(src, dst, w_sem.at[3 + n])

    other(4).start()
    x_copy(0).start()
    x_copy(1).start()
    for j in range(3):
        wqkv_copy(j).start()
    x_copy(2).start()
    x_copy(3).start()
    zs[0] = 0

    hh = lax.broadcasted_iota(jnp.int32, (H, D), 0)
    cc = lax.broadcasted_iota(jnp.int32, (H, D), 1)
    inhead = (cc >= hh * DH) & (cc < hh * DH + DH)
    expand = jnp.where(inhead, 1.0, 0.0).astype(bf16)
    dcol = jnp.sum(jnp.where(inhead, cc - hh * DH, 0), axis=0, keepdims=True)

    def xyz_pattern(r):
        j = r >> 3
        p = (r >> 1) & 3
        par = r & 1
        f = jnp.where(p == j, 16 + j, 16 + p - jnp.where(p > j, 1, 0))
        hl = jnp.where(p == j, 6 + par, 2 * j + par)
        return f, hl

    r = lax.broadcasted_iota(jnp.int32, (56, DH), 0)
    j = lax.broadcasted_iota(jnp.int32, (56, DH), 1)
    frow = jnp.where(r < 32, r >> 1, xyz_pattern(r & 31)[0])
    a0 = jnp.where(frow == j, 1.0, jnp.where(j == DH - 1, -1.0, 0.0)).astype(bf16)
    other(4).wait()
    t0 = jnp.zeros((DH, D), f32)
    for d in range(DH):
        t0 = jnp.where(dcol == d, _mm(wphi_v[d], expand), t0)
    t0 = _mm(a0, t0.astype(bf16)) * LOG2E

    blocks = []
    for q in range(4):
        for g in range(4):
            blocks.append((q, g))
            if g == 3 - q:
                blocks.append((q, 4))

    def tiles_of(q, kind):
        if kind == 4 or kind == 3 - q:
            return (q, q + 1)
        return (q,) if kind < 3 - q else (q + 1,)

    r = lax.broadcasted_iota(jnp.int32, (32, 128), 0)
    c = lax.broadcasted_iota(jnp.int32, (32, 128), 1)
    col_g = c - (r & 1) * DH
    col_x = (c - xyz_pattern(r)[1] * DH)[0:24]
    pts = []
    for t in range(5):
        mine = [b for b in blocks if t in tiles_of(*b)]
        parts = []
        for q, kind in mine:
            if kind == 4:
                rel, src = col_x + (128 * t - 160 * q), t0[32:56, 128 * t:128 * (t + 1)]
            else:
                rel, src = col_g + (128 * t - 160 * q - GR * kind), t0[0:32, 128 * t:128 * (t + 1)]
            parts.append(jnp.where((rel >= 0) & (rel < DH), src, 0.0))
        pts.append((mine, _cat(0, *parts).astype(bf16)))

    def prep_chunk(c):
        o, n = WCHUNKS[c]
        rows = slice(o * 128, (o + n) * 128)
        wall[WROW[2] // 2:(WROW[2] + D) // 2, rows] = _pk(wqkv_v[rows, 2 * D:3 * D].T)
        for j in (1, 0):
            res = {}
            for t, (mine, pt) in enumerate(pts):
                out = _mm_nt(pt, wqkv_v[rows, j * D + 128 * t:j * D + 128 * (t + 1)])
                o2 = 0
                for b in mine:
                    nb = 24 if b[1] == 4 else 32
                    blk = out[o2:o2 + nb]
                    o2 += nb
                    res[b] = blk if b not in res else res[b] + blk
            parts = []
            for q in range(4):
                parts += [res[(q, k)] for k in (4, 0, 1, 2, 3)]
            wall[WROW[j] // 2:(WROW[j] + DP) // 2, rows] = _pk(_cat(0, *parts).astype(bf16))

    def halves(j):
        hh_ = WLEN[j] // 2
        return (slice(WROW[j] // 2, (WROW[j] + hh_) // 2), slice((WROW[j] + hh_) // 2, (WROW[j] + 2 * hh_) // 2),
                slice(HROW[j] // 2, (HROW[j] + hh_) // 2))

    def wcomb(j, ks, tl):
        top, bot, cr = halves(j)
        lo, hi = slice(128 * tl, 128 * (tl + 1)), slice(256 + 128 * tl, 256 + 128 * (tl + 1))

        def ld(r_, c_):
            return _upk(wall[r_, c_]).astype(f32)

        for k in ks:
            v = (lambda: ld(top, lo) + ld(bot, hi), lambda: ld(bot, lo) + ld(bot, hi), lambda: ld(top, lo) + ld(top, hi),
                 lambda: ld(bot, lo) - ld(top, lo), lambda: ld(top, hi) - ld(bot, hi))[k]()
            wcmb[cr, 256 * k + 128 * tl:256 * k + 128 * (tl + 1)] = _pk(v.astype(bf16))

    def proj_part(j, k0, k1):
        cols = slice(k0 * 128, k1 * 128)
        rows = slice(WROW[j], WROW[j] + WLEN[j])
        part = _mm_nt(_upk(wall[WROW[j] // 2:(WROW[j] + WLEN[j]) // 2, cols]), _upk(xn01[:, cols]))
        if k0 > 0:
            part = part + acc_s[rows, :]
        acc_s[rows, :] = part

    def ldx(off, n):
        return x_v[pl.ds(off, n), :].astype(f32)

    def ln_next(off):
        wall[XROW:XROW + AR // 2, :] = _pk(_layernorm(ldx(off, AR)).astype(bf16))
        xn_v[...] = _pk(_layernorm(ldx(off + AR, SB - AR)).astype(bf16))

    def sq(pq, off, g0):
        for g, lg in enumerate(_group_logits(pq)):
            phiq[40 * (g0 + g):40 * (g0 + g + 1), pl.ds(off, pq.shape[1])] = _pk(_dual_softmax(lg, (g0 + g) % 3 == 1))

    def sk(pk, c0, g0):
        for g, lg in enumerate(_group_logits(pk)):
            phik_s[40 * (g0 + g):40 * (g0 + g + 1), c0:c0 + pk.shape[1]] = _pk(_dual_softmax(lg, (g0 + g) % 3 == 1))

    def sv(pv, slot):
        T = pv.shape[1]
        low = lax.broadcasted_iota(jnp.int32, (8, T), 0) < 4
        cols = slice(slot * SB, slot * SB + T)
        for t in range(5):
            mid = pv[120 * t + 56:120 * t + 64]
            blk = _cat(0, pv[120 * t:120 * t + 56], jnp.where(low, mid, 1.0), jnp.where(low, 1.0, mid),
                       pv[120 * t + 64:120 * t + 120])
            vext_s[64 * t:64 * (t + 1), cols] = _pk(blk.astype(bf16))
        vext_s[320:344, cols] = _pk(_cat(0, pv[600:640], jnp.ones((8, T), f32)).astype(bf16))

    def kv(slot, first=False, nslot=1):
        cols = slice(slot * SB, (slot + nslot) * SB)
        for r0, nr, f0, nf in TILES:
            upd = _mm_nt(_upk(vext_s[r0 // 2:(r0 + nr) // 2, cols]), _upk(phik_s[f0 // 2:(f0 + nf) // 2, cols]))
            if first:
                kvt[r0:r0 + nr, 0:nf] = upd
            else:
                kvt[r0:r0 + nr, 0:nf] += upd

    def sprod(j, p, t, anchor):
        top, bot, cr = halves(j)
        if p == 3 and anchor:
            lhs = _cat(0, wall[pl.ds(pl.multiple_of(zs[0] + top.start, 8), 8), 0:256],
                       wall[top.start + 8:top.stop, 0:256])
        elif p == 3:
            lhs = wall[top, 0:256]
        elif p == 4:
            lhs = wall[bot, 256:512]
        elif p == 1:
            lhs = wcmb[cr, 0:256]
        else:
            k, rem = {2: (1, bot), 5: (2, top), 6: (3, bot), 7: (4, top)}[p]
            lhs = _cat(1, wcmb[cr, 256 * k:256 * (k + 1)], wall[rem, 512:D])
        return _mm_nt(_upk(lhs), t[p])

    def pair(xa, off, noff):
        t = [{}, {}]
        m = {}
        pv = {}

        def put(p, v):
            for n_ in range(2):
                t[n_][p] = v[128 * n_:128 * (n_ + 1)].astype(bf16)

        def emit(j, half, sub, n_, val):
            if j == 1:
                sk(val, sub * SB + 128 * n_, 8 * half)
            elif j == 0:
                sq(val, off + sub * SB + 128 * n_, 8 * half)
            else:
                pv[half, sub, n_] = val

        def step(j, p, n_):
            v = sprod(j, p, t[n_], (j, p, n_) == (1, 3, 0))
            if p in (5, 2):
                m[j, p, n_] = v
            elif p == 1:
                m[j, 22, n_] = v - m[j, 2, n_]
                m[j, 11, n_] = v - m[j, 5, n_]
            elif p == 3:
                emit(j, 0, 1, n_, v + m[j, 5, n_])
                m[j, 22, n_] = m[j, 22, n_] + v
            elif p == 4:
                emit(j, 1, 0, n_, v + m[j, 2, n_])
                m[j, 11, n_] = m[j, 11, n_] + v
            elif p == 7:
                emit(j, 0, 0, n_, m[j, 11, n_] + v)
            else:
                emit(j, 1, 1, n_, m[j, 22, n_] + v)

        def pvs(sub):
            return _cat(0, *[_cat(1, pv[h_, sub, 0], pv[h_, sub, 1]) for h_ in range(2)])

        b11, b21, r1 = xa[:, 0:256], xa[:, 256:512], xa[:, 512:D]
        put(2, _cat(1, b11, r1))
        put(4, b21 - b11)
        for j in (1, 0, 2):
            step(j, 2, 0)
            step(j, 2, 1)
        xb = _layernorm(ldx(off + SB, SB))
        b12, b22, r2 = xb[:, 0:256], xb[:, 256:512], xb[:, 512:D]
        r12 = r1 + r2
        put(5, xb[:, 256:D])
        put(3, b12 - b22)
        put(1, b11 + b22)
        put(6, _cat(1, b11 + b12, r12))
        put(7, _cat(1, b21 + b22, r12))
        for p in (5, 1):
            step(1, p, 0)
            step(1, p, 1)
        ln_next(noff)
        seq = (((1, 3), (0, 5)), ((1, 4), (2, 5)), ((1, 7), (0, 1)), ((1, 6), (2, 1)),
               ((0, 3), (2, 3)), ((0, 4), (2, 4)), ((0, 7), (2, 7)), ((0, 6), (2, 6)))
        for k_, (sdot, fdot) in enumerate(seq):
            if k_ == 7:
                sv(pvs(0), 0)
            for n_ in range(2):
                step(*sdot, n_)
                step(*fdot, n_)
        kv(0)
        sv(pvs(1), 1)
        kv(1)

    x_copy(0).wait()
    x_copy(1).wait()
    xn01[...] = _pk(_layernorm(ldx(0, 2 * SB)).astype(bf16))
    wqkv_copy(0).wait()
    prep_chunk(0)
    for j in (2, 1, 0):
        wcomb(j, (3,), 0)
    for j in (2, 1, 0):
        proj_part(j, 0, 1)
    wqkv_copy(1).wait()
    prep_chunk(1)
    for j in (2, 1, 0):
        wcomb(j, (3,), 1)
        wcomb(j, (0, 1, 2, 4), 0)
    proj_part(2, 1, 3)
    proj_part(1, 1, 2)
    proj_part(0, 1, 2)
    wqkv_copy(2).wait()
    x_copy(2).wait()
    for n in range(4):
        other(n).start()
    prep_chunk(2)
    for j in (2, 1, 0):
        wcomb(j, (0, 1, 2, 4), 1)

    un = [(u, n_) for u in range(2) for n_ in range(4)]
    pv01 = {}

    def fin01(j, u, n_):
        r0 = WROW[j] + u * (DP // 2)
        part = _mm_nt(_upk(wall[r0 // 2:(r0 + DP // 2) // 2, 256:D]), _upk(xn01[64 * n_:64 * (n_ + 1), 256:D]))
        part = part + acc_s[r0:r0 + DP // 2, 128 * n_:128 * (n_ + 1)]
        if j == 1:
            sk(part, 2 * SB + 128 * n_, 8 * u)
        else:
            sq(part, 128 * n_, 8 * u)

    def vunit(k_):
        u, n_ = un[k_ // 2]
        kt = 3 + k_ % 2
        r0 = WROW[2] + u * (D // 2)
        prev = acc_s[r0:r0 + D // 2, 128 * n_:128 * (n_ + 1)] if kt == 3 else pv01[u, n_]
        pv01[u, n_] = prev + _mm_nt(_upk(wall[r0 // 2:(r0 + D // 2) // 2, 128 * kt:128 * (kt + 1)]),
                                    _upk(xn01[64 * n_:64 * (n_ + 1), 128 * kt:128 * (kt + 1)]))

    for k_ in range(4):
        vunit(k_)
    for k_ in range(16):
        fin01(1 - k_ // 8, *un[k_ % 8])
        if k_ < 12:
            vunit(4 + k_)
        if k_ == 11:
            sv(_cat(0, *[_cat(1, *[pv01[u, n_] for n_ in range(4)]) for u in range(2)]), 2)
            ln_next(2 * SB)
    kv(2, first=True, nslot=2)
    x_copy(3).wait()

    def phase1(i, carry):
        off = pl.multiple_of((2 + i * 2) * SB, SB)
        noff = pl.multiple_of(jnp.minimum(4 + i * 2, NSUB - 1) * SB, SB)
        pair(_upk(_cat(0, wall[XROW:XROW + AR // 2, :], xn_v[...])).astype(f32), off, noff)
        return carry

    lax.fori_loop(0, NSUB // 2 - 1, phase1, 0)

    r = lax.broadcasted_iota(jnp.int32, (64, 128), 0)
    c = lax.broadcasted_iota(jnp.int32, (64, 128), 1)

    def third(v):
        return jnp.where(v < DH, 0, jnp.where(v < GR, 1, 2))

    m_a = jnp.where(r < 60, third(r), jnp.minimum(r - 60, 2)) == jnp.where(c < 80, c & 1, jnp.where(c < 120, 2, 3))
    m_b = jnp.where(r < 4, jnp.minimum(r, 2), third(r - 4)) == jnp.where(c < 8, 3, jnp.where(c < 48, 0, 1 + (c & 1)))
    m_c = (jnp.where(r < GR, third(r), jnp.where(r < GR + 4, 0, 1)) == (c & 1))[0:48, 0:80]
    for b, (r0, nr, f0, nf) in enumerate(TILES):
        m = m_c if b == 10 else (m_a, m_b)[b % 2]
        lmat[r0 // 2:(r0 + nr) // 2, 0:nf] = _pk(jnp.where(m, kvt[r0:r0 + nr, 0:nf], 0.0).astype(bf16))

    for n in range(4):
        other(n).wait()

    def phase2(i, carry):
        off = pl.multiple_of(i * (2 * SB), 2 * SB)
        low = lax.broadcasted_iota(jnp.int32, (8, SB), 0) < 4
        ots = []
        for s in range(2):
            parts = []
            ogs = [_mm(_upk(lmat[r0 // 2:(r0 + nr) // 2, 0:nf]),
                       _upk(phiq[f0 // 2:(f0 + nf) // 2, pl.ds(off + s * SB, SB)])) for r0, nr, f0, nf in TILES]
            for t in range(5):
                oa, ob = ogs[2 * t], ogs[2 * t + 1]
                rc = _recip(jnp.where(low, ob[0:8], oa[56:64]) + 1e-6)
                bc = [jnp.broadcast_to(rc[k:k + 1], (8, SB)) for k in (4, 5, 6, 0, 1, 2)]
                parts += [oa[0:8] * bc[0], oa[8:16] * bc[0], oa[16:24] * jnp.where(low, bc[0], bc[1]),
                          oa[24:32] * bc[1], oa[32:40] * bc[1], oa[40:48] * bc[2], oa[48:56] * bc[2],
                          jnp.where(low, oa[56:64], ob[0:8]) * jnp.where(low, bc[2], bc[3]),
                          ob[8:16] * bc[3], ob[16:24] * bc[3], ob[24:32] * bc[4], ob[32:40] * bc[4],
                          ob[40:48] * jnp.where(low, bc[4], bc[5]), ob[48:56] * bc[5], ob[56:64] * bc[5]]
            og = ogs[10]
            rc = _recip(og[40:48] + 1e-6)
            rr = pltpu.roll(rc, 4, 0)
            r0_ = jnp.where(low, rc, rr)
            r1_ = jnp.where(low, rr, rc)
            parts += [og[0:8] * r0_, og[8:16] * r0_, og[16:24] * rc, og[24:32] * r1_, og[32:40] * r1_]
            ots.append(_cat(0, *parts).astype(bf16))
        hs = []
        for s in range(2):
            h = ldx(off + s * SB, SB) + lax.dot_general(ots[s], wo_v[...], TN, preferred_element_type=f32)
            hs.append((h, _layernorm(h)))

        ha, hb = hs[0][1], hs[1][1]
        a11, a12, a21, a22 = ha[:, 0:256], ha[:, 256:512], hb[:, 0:256], hb[:, 256:512]
        ra, rb = ha[:, 512:D], hb[:, 512:D]
        s1, s2r, s3, s4, s5r, s6r, s7r = [v.astype(bf16) for v in (
            a11 + a22, _cat(1, a21 + a22, rb), a11, a22, _cat(1, a11 + a12, ra), _cat(1, a21 - a11, rb),
            _cat(1, a12 - a22, ra))]

        def wcols(r0, r1, c0):
            return _cat(1, wg_v[r0:r1, c0:c0 + CW], wu_v[r0:r1, c0:c0 + CW])

        def wcols32(r0, r1, c0):
            return _cat(1, wg_v[r0:r1, c0:c0 + CW].astype(f32), wu_v[r0:r1, c0:c0 + CW].astype(f32))

        def glu(c):
            return jax.nn.gelu(c[:, 0:CW], approximate=True) * c[:, CW:2 * CW]

        m5s = [_mm(s5r, wcols(256, D, HF + c * CW)) for c in range(NA)]
        for c in range(NCH):
            c1, c2 = c * CW, HF + c * CW
            f11, f12, f21, f22 = wcols32(0, 256, c1), wcols32(0, 256, c2), wcols32(256, 512, c1), wcols32(256, 512, c2)
            r12 = wcols32(512, D, c1) + wcols32(512, D, c2)
            m5 = m5s[c] if c < NA else _mm(s5r, wcols(256, D, c2))
            m2 = _mm(s2r, _cat(0, wcols(0, 256, c1), wcols(512, D, c1)))
            m1 = _mm(s1, (f11 + f22).astype(bf16))
            p22 = m1 - m2
            p11 = m1 - m5
            m3 = _mm(s3, (f12 - f22).astype(bf16))
            c12 = m3 + m5
            p22 = p22 + m3
            m4 = _mm(s4, (f21 - f11).astype(bf16))
            c21 = m2 + m4
            p11 = p11 + m4
            c11 = p11 + _mm(s7r, _cat(0, f21 + f22, r12).astype(bf16))
            c22 = p22 + _mm(s6r, _cat(0, f11 + f12, r12).astype(bf16))
            q11, q12, q21, q22 = glu(c11), glu(c12), glu(c21), glu(c22)
            for k, v in enumerate((q11 + q22, q21 + q22, q11, q22, q11 + q12, q21 - q11, q12 - q22, q12, q21)):
                d_s[:, k * HF + c * CW:k * HF + (c + 1) * CW] = _pk(v.astype(bf16))

        def dn_rhs(k0, k1):
            f11, f12 = wd_v[k0:k1, 0:256].astype(f32), wd_v[k0:k1, 256:512].astype(f32)
            f21, f22 = wd_v[HF + k0:HF + k1, 0:256].astype(f32), wd_v[HF + k0:HF + k1, 256:512].astype(f32)
            w4 = _cat(0, wd_v[k0:k1, 512:D], wd_v[HF + k0:HF + k1, 512:D])
            return [(f11 + f22).astype(bf16), wd_v[k0:k1, 0:256], (f12 - f22).astype(bf16), (f21 - f11).astype(bf16),
                    wd_v[HF + k0:HF + k1, 256:512], (f11 + f12).astype(bf16), (f21 + f22).astype(bf16), w4, w4]

        def dn_stage(ya, yb, r0, r1, k0, k1, t, done=None):
            rows = slice(r0 // 2, r1 // 2)

            def f(k):
                if k < 7:
                    return _mm(_upk(d_s[rows, k * HF + k0:k * HF + k1]), t[k])
                lo, hi = ((2, 7), (8, 3))[k - 7]
                return _mm(_upk(_cat(1, d_s[rows, lo * HF + k0:lo * HF + k1], d_s[rows, hi * HF + k0:hi * HF + k1])),
                           t[k])

            a4 = ya[:, 512:D] + f(7)
            m5, m2, m1 = f(4), f(1), f(0)
            p11 = ya[:, 0:256] + m1 - m5
            p22 = yb[:, 256:512] + m1 - m2
            m3 = f(2)
            c12 = ya[:, 256:512] + m5 + m3
            p22 = p22 + m3
            m4 = f(3)
            c21 = yb[:, 0:256] + m2 + m4
            p11 = p11 + m4
            ya = _cat(1, p11 + f(6), c12, a4)
            if done is not None:
                done(0, ya)
            b4 = yb[:, 512:D] + f(8)
            yb = _cat(1, c21, p22 + f(5), b4)
            if done is not None:
                done(1, yb)
            return ya, yb

        ya, yb = dn_stage(hs[0][0], hs[1][0], 0, SB, 0, KD, dn_rhs(0, KD))
        t = dn_rhs(KD, HF)
        r0 = 0
        for nr in CH:
            def done(s_, y):
                rows = pl.ds(off + s_ * SB + r0, nr)
                out_v[rows, :] = y.astype(bf16)
                pltpu.make_async_copy(out_v.at[rows], out_hbm.at[rows], o_sem.at[0]).start()

            dn_stage(ya[r0:r0 + nr], yb[r0:r0 + nr], r0, r0 + nr, KD, HF, t, done)
            r0 += nr
        return carry

    lax.fori_loop(0, NSUB // 2, phase2, 0)
    pltpu.make_async_copy(out_v, out_hbm, o_sem.at[0]).wait()


def _compiler_params():
    try:
        return pltpu.CompilerParams(vmem_limit_bytes=100 * 1024 * 1024, disable_bounds_checks=True,
                                    disable_semaphore_checks=True)
    except TypeError:
        return pltpu.CompilerParams(vmem_limit_bytes=100 * 1024 * 1024)


@jax.jit
def pallas_sequential_preLN__linear_kernel_hedgehog__geglu_ffn__prompt_kernel(
    A_x: jax.Array,
    A_wqkv: jax.Array,
    A_w_phi: jax.Array,
    A_wo: jax.Array,
    B_x: jax.Array,
    B_w_gate: jax.Array,
    B_w_up: jax.Array,
    B_w_down: jax.Array,
):
    x = A_x.reshape(S, D)
    wphi_t = jnp.transpose(A_w_phi, (1, 2, 0))
    anyspec = pl.BlockSpec(memory_space=pl.ANY)
    out = pl.pallas_call(
        _kernel,
        out_shape=jax.ShapeDtypeStruct((S, D), bf16),
        in_specs=[anyspec] * 7,
        out_specs=anyspec,
        scratch_shapes=[
            pltpu.VMEM((S, D), bf16),
            pltpu.VMEM((D, 3 * D), bf16),
            pltpu.VMEM((DH, DH, H), bf16),
            pltpu.VMEM((D, D), bf16),
            pltpu.VMEM((D, F), bf16),
            pltpu.VMEM((D, F), bf16),
            pltpu.VMEM((F, D), bf16),
            pltpu.VMEM((S, D), bf16),
            pltpu.SMEM((1,), jnp.int32),
            pltpu.VMEM(((SB - AR) // 2, D), u32),
            pltpu.VMEM((SB, D), u32),
            pltpu.VMEM((2 * DP + D, 2 * SB), f32),
            pltpu.VMEM((XROW + AR // 2, D), u32),
            pltpu.VMEM(((2 * DP + D) // 4, 5 * 256), u32),
            pltpu.VMEM((NG * 40, S), u32),
            pltpu.VMEM((NG * 40, 4 * SB), u32),
            pltpu.VMEM((344, 4 * SB), u32),
            pltpu.VMEM((688, 128), f32),
            pltpu.VMEM((344, 128), u32),
            pltpu.VMEM((SB // 2, 9 * HF), u32),
            pltpu.SemaphoreType.DMA((4,)),
            pltpu.SemaphoreType.DMA((8,)),
            pltpu.SemaphoreType.DMA((1,)),
        ],
        compiler_params=_compiler_params(),
    )(x, A_wqkv, wphi_t, A_wo, B_w_gate, B_w_up, B_w_down)
    return out.reshape(1, S, D)
```

```python
import jax
import jax.numpy as jnp
from jax import lax
import jax.experimental.pallas as pl
import jax.experimental.pallas.tpu as pltpu

S, D, H, DH, F = 2048, 640, 32, 20, 1536
NG = H // 2
GR = 2 * DH
DP = H * (DH - 1)
HF = F // 2
LOG2E = 1.4426950408889634
NT = (((1,), (1,)), ((), ()))
TN = (((0,), (0,)), ((), ()))
f32 = jnp.float32
bf16 = jnp.bfloat16
u32 = jnp.uint32
SB = 256
NSUB = S // SB
WROW = (0, DP, 2 * DP)
WLEN = (DP, DP, D)
HROW = (0, DP // 2, DP)
XROW = (2 * DP + D) // 2
TILES = [(64 * b, 64, 240 * (b // 2) + 112 * (b % 2), 128) for b in range(10)] + [(640, 48, 1200, 80)]
XCHUNKS = [(0, SB), (SB, SB), (2 * SB, SB), (3 * SB, 5 * SB)]
WCHUNKS = [(0, 1), (1, 2), (3, 2)]
AR = 128
NCH = 3
CW = HF // NCH
NA = 2
KD = 512
CH = (128, 64, 64)


def _layernorm(x):
    m = jnp.mean(x, axis=-1, keepdims=True)
    xc = x - m
    v = jnp.mean(xc * xc, axis=-1, keepdims=True)
    return xc * lax.rsqrt(v + 1e-5)


def _recip(x):
    r = pl.reciprocal(x, approx=True)
    return r * (2.0 - x * r)


def _fold8(x, op):
    x = op(x, pltpu.roll(x, 2, 0))
    return op(x, pltpu.roll(x, 4, 0))


def _dual_softmax(p, split):
    T = p.shape[1]
    p3 = p.reshape(5, 8, T)
    mx = _fold8(jnp.max(p3, axis=0), jnp.maximum)
    mn = _fold8(jnp.min(p3, axis=0), jnp.minimum)
    ep = jnp.exp2(p3 - mx[None])
    en = jnp.exp2(mn[None] - p3)
    ep = ep * _recip(_fold8(jnp.sum(ep, axis=0), jnp.add))[None]
    en = en * _recip(_fold8(jnp.sum(en, axis=0), jnp.add))[None]
    if split:
        even = (lax.broadcasted_iota(jnp.int32, (5, 8, T), 1) & 1) == 0
        ep, en = (jnp.where(even, ep, pltpu.roll(en, 1, 1)), jnp.where(even, pltpu.roll(ep, 7, 1), en))
    return jnp.concatenate([ep, en], axis=0).reshape(2 * GR, T).astype(bf16)


def _group_logits(p):
    T = p.shape[1]
    pr = lax.broadcasted_iota(jnp.int32, (8, T), 0) >> 1
    out = []
    for q in range(p.shape[0] // 152):
        base = 152 * q
        xyz = [p[base + 8 * j:base + 8 * (j + 1)] for j in range(3)]
        last = [jnp.where(pr == j, 0.0, xyz[j]) for j in range(3)]
        last.append(jnp.where(pr == 0, xyz[0], jnp.where(pr == 1, xyz[1], jnp.where(pr == 2, xyz[2], 0.0))))
        for g in range(4):
            out.append(jnp.concatenate([last[g], p[base + 24 + 32 * g:base + 24 + 32 * (g + 1)]], axis=0))
    return out


def _pk(val):
    return pltpu.bitcast(val, u32)


def _upk(val):
    return pltpu.bitcast(val, bf16)


def _cat(axis, *vs):
    return jnp.concatenate(vs, axis=axis)


def _mm(x, y):
    return jnp.dot(x, y, preferred_element_type=f32)


def _mm_nt(x, y):
    return lax.dot_general(x, y, NT, preferred_element_type=f32)


def _kernel(x_hbm, wqkv_hbm, wphi_hbm, wo_hbm, wg_hbm, wu_hbm, wd_hbm, out_hbm,
            x_v, wqkv_v, wphi_v, wo_v, wg_v, wu_v, wd_v, out_v,
            zs, xn_v, xn01, acc_s, wall, wcmb, phiq, phik_s, vext_s, kvt, lmat, d_s, x_sem, w_sem, o_sem):

    def x_copy(i):
        o, n = XCHUNKS[i]
        return pltpu.make_async_copy(x_hbm.at[pl.ds(o, n)], x_v.at[pl.ds(o, n)], x_sem.at[i])

    def wqkv_copy(j):
        o, n = WCHUNKS[j]
        return pltpu.make_async_copy(wqkv_hbm.at[pl.ds(o * 128, n * 128)], wqkv_v.at[pl.ds(o * 128, n * 128)],
                                     w_sem.at[j])

    def other(n):
        src, dst = ((wo_hbm, wo_v), (wg_hbm, wg_v), (wu_hbm, wu_v), (wd_hbm, wd_v), (wphi_hbm, wphi_v))[n]
        return pltpu.make_async_copy(src, dst, w_sem.at[3 + n])

    other(4).start()
    x_copy(0).start()
    x_copy(1).start()
    for j in range(3):
        wqkv_copy(j).start()
    x_copy(2).start()
    x_copy(3).start()
    zs[0] = 0

    hh = lax.broadcasted_iota(jnp.int32, (H, D), 0)
    cc = lax.broadcasted_iota(jnp.int32, (H, D), 1)
    inhead = (cc >= hh * DH) & (cc < hh * DH + DH)
    expand = jnp.where(inhead, 1.0, 0.0).astype(bf16)
    dcol = jnp.sum(jnp.where(inhead, cc - hh * DH, 0), axis=0, keepdims=True)

    def xyz_pattern(r):
        j = r >> 3
        p = (r >> 1) & 3
        par = r & 1
        f = jnp.where(p == j, 16 + j, 16 + p - jnp.where(p > j, 1, 0))
        hl = jnp.where(p == j, 6 + par, 2 * j + par)
        return f, hl

    r = lax.broadcasted_iota(jnp.int32, (56, DH), 0)
    j = lax.broadcasted_iota(jnp.int32, (56, DH), 1)
    frow = jnp.where(r < 32, r >> 1, xyz_pattern(r & 31)[0])
    a0 = jnp.where(frow == j, 1.0, jnp.where(j == DH - 1, -1.0, 0.0)).astype(bf16)
    other(4).wait()
    t0 = jnp.zeros((DH, D), f32)
    for d in range(DH):
        t0 = jnp.where(dcol == d, _mm(wphi_v[d], expand), t0)
    t0 = _mm(a0, t0.astype(bf16)) * LOG2E

    blocks = []
    for q in range(4):
        for g in range(4):
            blocks.append((q, g))
            if g == 3 - q:
                blocks.append((q, 4))

    def tiles_of(q, kind):
        if kind == 4 or kind == 3 - q:
            return (q, q + 1)
        return (q,) if kind < 3 - q else (q + 1,)

    r = lax.broadcasted_iota(jnp.int32, (32, 128), 0)
    c = lax.broadcasted_iota(jnp.int32, (32, 128), 1)
    col_g = c - (r & 1) * DH
    col_x = (c - xyz_pattern(r)[1] * DH)[0:24]
    pts = []
    for t in range(5):
        mine = [b for b in blocks if t in tiles_of(*b)]
        parts = []
        for q, kind in mine:
            if kind == 4:
                rel, src = col_x + (128 * t - 160 * q), t0[32:56, 128 * t:128 * (t + 1)]
            else:
                rel, src = col_g + (128 * t - 160 * q - GR * kind), t0[0:32, 128 * t:128 * (t + 1)]
            parts.append(jnp.where((rel >= 0) & (rel < DH), src, 0.0))
        pts.append((mine, _cat(0, *parts).astype(bf16)))

    def prep_chunk(c):
        o, n = WCHUNKS[c]
        rows = slice(o * 128, (o + n) * 128)
        wall[WROW[2] // 2:(WROW[2] + D) // 2, rows] = _pk(wqkv_v[rows, 2 * D:3 * D].T)
        for j in (1, 0):
            res = {}
            for t, (mine, pt) in enumerate(pts):
                out = _mm_nt(pt, wqkv_v[rows, j * D + 128 * t:j * D + 128 * (t + 1)])
                o2 = 0
                for b in mine:
                    nb = 24 if b[1] == 4 else 32
                    blk = out[o2:o2 + nb]
                    o2 += nb
                    res[b] = blk if b not in res else res[b] + blk
            parts = []
            for q in range(4):
                parts += [res[(q, k)] for k in (4, 0, 1, 2, 3)]
            wall[WROW[j] // 2:(WROW[j] + DP) // 2, rows] = _pk(_cat(0, *parts).astype(bf16))

    def halves(j):
        hh_ = WLEN[j] // 2
        return (slice(WROW[j] // 2, (WROW[j] + hh_) // 2), slice((WROW[j] + hh_) // 2, (WROW[j] + 2 * hh_) // 2),
                slice(HROW[j] // 2, (HROW[j] + hh_) // 2))

    def wcomb(j, ks, tl):
        top, bot, cr = halves(j)
        lo, hi = slice(128 * tl, 128 * (tl + 1)), slice(256 + 128 * tl, 256 + 128 * (tl + 1))

        def ld(r_, c_):
            return _upk(wall[r_, c_]).astype(f32)

        for k in ks:
            v = (lambda: ld(top, lo) + ld(bot, hi), lambda: ld(bot, lo) + ld(bot, hi), lambda: ld(top, lo) + ld(top, hi),
                 lambda: ld(bot, lo) - ld(top, lo), lambda: ld(top, hi) - ld(bot, hi))[k]()
            wcmb[cr, 256 * k + 128 * tl:256 * k + 128 * (tl + 1)] = _pk(v.astype(bf16))

    def proj_part(j, k0, k1):
        cols = slice(k0 * 128, k1 * 128)
        rows = slice(WROW[j], WROW[j] + WLEN[j])
        part = _mm_nt(_upk(wall[WROW[j] // 2:(WROW[j] + WLEN[j]) // 2, cols]), _upk(xn01[:, cols]))
        if k0 > 0:
            part = part + acc_s[rows, :]
        acc_s[rows, :] = part

    def ldx(off, n):
        return x_v[pl.ds(off, n), :].astype(f32)

    def ln_next(off):
        wall[XROW:XROW + AR // 2, :] = _pk(_layernorm(ldx(off, AR)).astype(bf16))
        xn_v[...] = _pk(_layernorm(ldx(off + AR, SB - AR)).astype(bf16))

    def sq(pq, off, g0):
        for g, lg in enumerate(_group_logits(pq)):
            phiq[40 * (g0 + g):40 * (g0 + g + 1), pl.ds(off, pq.shape[1])] = _pk(_dual_softmax(lg, (g0 + g) % 3 == 1))

    def sk(pk, c0, g0):
        for g, lg in enumerate(_group_logits(pk)):
            phik_s[40 * (g0 + g):40 * (g0 + g + 1), c0:c0 + pk.shape[1]] = _pk(_dual_softmax(lg, (g0 + g) % 3 == 1))

    def sv(pv, slot):
        T = pv.shape[1]
        low = lax.broadcasted_iota(jnp.int32, (8, T), 0) < 4
        cols = slice(slot * SB, slot * SB + T)
        for t in range(5):
            mid = pv[120 * t + 56:120 * t + 64]
            blk = _cat(0, pv[120 * t:120 * t + 56], jnp.where(low, mid, 1.0), jnp.where(low, 1.0, mid),
                       pv[120 * t + 64:120 * t + 120])
            vext_s[64 * t:64 * (t + 1), cols] = _pk(blk.astype(bf16))
        vext_s[320:344, cols] = _pk(_cat(0, pv[600:640], jnp.ones((8, T), f32)).astype(bf16))

    def kv(slot, first=False, nslot=1):
        cols = slice(slot * SB, (slot + nslot) * SB)
        for r0, nr, f0, nf in TILES:
            upd = _mm_nt(_upk(vext_s[r0 // 2:(r0 + nr) // 2, cols]), _upk(phik_s[f0 // 2:(f0 + nf) // 2, cols]))
            if first:
                kvt[r0:r0 + nr, 0:nf] = upd
            else:
                kvt[r0:r0 + nr, 0:nf] += upd

    def sprod(j, p, t, anchor):
        top, bot, cr = halves(j)
        if p == 3 and anchor:
            lhs = _cat(0, wall[pl.ds(pl.multiple_of(zs[0] + top.start, 8), 8), 0:256],
                       wall[top.start + 8:top.stop, 0:256])
        elif p == 3:
            lhs = wall[top, 0:256]
        elif p == 4:
            lhs = wall[bot, 256:512]
        elif p == 1:
            lhs = wcmb[cr, 0:256]
        else:
            k, rem = {2: (1, bot), 5: (2, top), 6: (3, bot), 7: (4, top)}[p]
            lhs = _cat(1, wcmb[cr, 256 * k:256 * (k + 1)], wall[rem, 512:D])
        return _mm_nt(_upk(lhs), t[p])

    def pair(xa, off, noff):
        t = [{}, {}]
        m = {}
        pv = {}

        def put(p, v):
            for n_ in range(2):
                t[n_][p] = v[128 * n_:128 * (n_ + 1)].astype(bf16)

        def emit(j, half, sub, n_, val):
            if j == 1:
                sk(val, sub * SB + 128 * n_, 8 * half)
            elif j == 0:
                sq(val, off + sub * SB + 128 * n_, 8 * half)
            else:
                pv[half, sub, n_] = val

        def step(j, p, n_):
            v = sprod(j, p, t[n_], (j, p, n_) == (1, 3, 0))
            if p in (5, 2):
                m[j, p, n_] = v
            elif p == 1:
                m[j, 22, n_] = v - m[j, 2, n_]
                m[j, 11, n_] = v - m[j, 5, n_]
            elif p == 3:
                emit(j, 0, 1, n_, v + m[j, 5, n_])
                m[j, 22, n_] = m[j, 22, n_] + v
            elif p == 4:
                emit(j, 1, 0, n_, v + m[j, 2, n_])
                m[j, 11, n_] = m[j, 11, n_] + v
            elif p == 7:
                emit(j, 0, 0, n_, m[j, 11, n_] + v)
            else:
                emit(j, 1, 1, n_, m[j, 22, n_] + v)

        def pvs(sub):
            return _cat(0, *[_cat(1, pv[h_, sub, 0], pv[h_, sub, 1]) for h_ in range(2)])

        b11, b21, r1 = xa[:, 0:256], xa[:, 256:512], xa[:, 512:D]
        put(2, _cat(1, b11, r1))
        put(4, b21 - b11)
        for j in (1, 0, 2):
            step(j, 2, 0)
            step(j, 2, 1)
        xb = _layernorm(ldx(off + SB, SB))
        b12, b22, r2 = xb[:, 0:256], xb[:, 256:512], xb[:, 512:D]
        r12 = r1 + r2
        put(5, xb[:, 256:D])
        put(3, b12 - b22)
        put(1, b11 + b22)
        put(6, _cat(1, b11 + b12, r12))
        put(7, _cat(1, b21 + b22, r12))
        for p in (5, 1):
            step(1, p, 0)
            step(1, p, 1)
        ln_next(noff)
        seq = (((1, 3), (0, 5)), ((1, 4), (2, 5)), ((1, 7), (0, 1)), ((1, 6), (2, 1)),
               ((0, 3), (2, 3)), ((0, 4), (2, 4)), ((0, 7), (2, 7)), ((0, 6), (2, 6)))
        for k_, (sdot, fdot) in enumerate(seq):
            if k_ == 7:
                sv(pvs(0), 0)
            for n_ in range(2):
                step(*sdot, n_)
                step(*fdot, n_)
        kv(0)
        sv(pvs(1), 1)
        kv(1)

    x_copy(0).wait()
    x_copy(1).wait()
    xn01[...] = _pk(_layernorm(ldx(0, 2 * SB)).astype(bf16))
    wqkv_copy(0).wait()
    prep_chunk(0)
    for j in (2, 1, 0):
        wcomb(j, (3,), 0)
    for j in (2, 1, 0):
        proj_part(j, 0, 1)
    wqkv_copy(1).wait()
    prep_chunk(1)
    for j in (2, 1, 0):
        wcomb(j, (3,), 1)
        wcomb(j, (0, 1, 2, 4), 0)
    proj_part(2, 1, 3)
    proj_part(1, 1, 2)
    proj_part(0, 1, 2)
    wqkv_copy(2).wait()
    x_copy(2).wait()
    for n in range(4):
        other(n).start()
    prep_chunk(2)
    for j in (2, 1, 0):
        wcomb(j, (0, 1, 2, 4), 1)

    un = [(u, n_) for u in range(2) for n_ in range(4)]
    pv01 = {}

    def fin01(j, u, n_):
        r0 = WROW[j] + u * (DP // 2)
        part = _mm_nt(_upk(wall[r0 // 2:(r0 + DP // 2) // 2, 256:D]), _upk(xn01[64 * n_:64 * (n_ + 1), 256:D]))
        part = part + acc_s[r0:r0 + DP // 2, 128 * n_:128 * (n_ + 1)]
        if j == 1:
            sk(part, 2 * SB + 128 * n_, 8 * u)
        else:
            sq(part, 128 * n_, 8 * u)

    def vunit(k_):
        u, n_ = un[k_ // 2]
        kt = 3 + k_ % 2
        r0 = WROW[2] + u * (D // 2)
        prev = acc_s[r0:r0 + D // 2, 128 * n_:128 * (n_ + 1)] if kt == 3 else pv01[u, n_]
        pv01[u, n_] = prev + _mm_nt(_upk(wall[r0 // 2:(r0 + D // 2) // 2, 128 * kt:128 * (kt + 1)]),
                                    _upk(xn01[64 * n_:64 * (n_ + 1), 128 * kt:128 * (kt + 1)]))

    for k_ in range(4):
        vunit(k_)
    for k_ in range(16):
        fin01(1 - k_ // 8, *un[k_ % 8])
        if k_ < 12:
            vunit(4 + k_)
        if k_ == 11:
            sv(_cat(0, *[_cat(1, *[pv01[u, n_] for n_ in range(4)]) for u in range(2)]), 2)
            ln_next(2 * SB)
    kv(2, first=True, nslot=2)
    x_copy(3).wait()

    def phase1(i, carry):
        off = pl.multiple_of((2 + i * 2) * SB, SB)
        noff = pl.multiple_of(jnp.minimum(4 + i * 2, NSUB - 1) * SB, SB)
        pair(_upk(_cat(0, wall[XROW:XROW + AR // 2, :], xn_v[...])).astype(f32), off, noff)
        return carry

    lax.fori_loop(0, NSUB // 2 - 1, phase1, 0)

    r = lax.broadcasted_iota(jnp.int32, (64, 128), 0)
    c = lax.broadcasted_iota(jnp.int32, (64, 128), 1)

    def third(v):
        return jnp.where(v < DH, 0, jnp.where(v < GR, 1, 2))

    m_a = jnp.where(r < 60, third(r), jnp.minimum(r - 60, 2)) == jnp.where(c < 80, c & 1, jnp.where(c < 120, 2, 3))
    m_b = jnp.where(r < 4, jnp.minimum(r, 2), third(r - 4)) == jnp.where(c < 8, 3, jnp.where(c < 48, 0, 1 + (c & 1)))
    m_c = (jnp.where(r < GR, third(r), jnp.where(r < GR + 4, 0, 1)) == (c & 1))[0:48, 0:80]
    for b, (r0, nr, f0, nf) in enumerate(TILES):
        m = m_c if b == 10 else (m_a, m_b)[b % 2]
        lmat[r0 // 2:(r0 + nr) // 2, 0:nf] = _pk(jnp.where(m, kvt[r0:r0 + nr, 0:nf], 0.0).astype(bf16))

    for n in range(4):
        other(n).wait()

    def phase2(i, carry):
        off = pl.multiple_of(i * (2 * SB), 2 * SB)
        low = lax.broadcasted_iota(jnp.int32, (8, SB), 0) < 4
        ots = []
        for s in range(2):
            parts = []
            ogs = [_mm(_upk(lmat[r0 // 2:(r0 + nr) // 2, 0:nf]),
                       _upk(phiq[f0 // 2:(f0 + nf) // 2, pl.ds(off + s * SB, SB)])) for r0, nr, f0, nf in TILES]
            for t in range(5):
                oa, ob = ogs[2 * t], ogs[2 * t + 1]
                rc = _recip(jnp.where(low, ob[0:8], oa[56:64]) + 1e-6)
                bc = [jnp.broadcast_to(rc[k:k + 1], (8, SB)) for k in (4, 5, 6, 0, 1, 2)]
                parts += [oa[0:8] * bc[0], oa[8:16] * bc[0], oa[16:24] * jnp.where(low, bc[0], bc[1]),
                          oa[24:32] * bc[1], oa[32:40] * bc[1], oa[40:48] * bc[2], oa[48:56] * bc[2],
                          jnp.where(low, oa[56:64], ob[0:8]) * jnp.where(low, bc[2], bc[3]),
                          ob[8:16] * bc[3], ob[16:24] * bc[3], ob[24:32] * bc[4], ob[32:40] * bc[4],
                          ob[40:48] * jnp.where(low, bc[4], bc[5]), ob[48:56] * bc[5], ob[56:64] * bc[5]]
            og = ogs[10]
            rc = _recip(og[40:48] + 1e-6)
            rr = pltpu.roll(rc, 4, 0)
            r0_ = jnp.where(low, rc, rr)
            r1_ = jnp.where(low, rr, rc)
            parts += [og[0:8] * r0_, og[8:16] * r0_, og[16:24] * rc, og[24:32] * r1_, og[32:40] * r1_]
            ots.append(_cat(0, *parts))

        def tn(x, y):
            return lax.dot_general(x.astype(bf16), y, TN, preferred_element_type=f32)

        oa, ob = ots
        o11, o12, o21, o22, ora, orb = oa[0:256], oa[256:512], ob[0:256], ob[256:512], oa[512:D], ob[512:D]
        g11, g12 = wo_v[0:256, 0:256].astype(f32), wo_v[0:256, 256:512].astype(f32)
        g21, g22 = wo_v[256:512, 0:256].astype(f32), wo_v[256:512, 256:512].astype(f32)
        gr = wo_v[512:D, 0:256].astype(f32) + wo_v[512:D, 256:512].astype(f32)
        xa, xb = ldx(off, SB), ldx(off + SB, SB)
        m3 = tn(o11, (g12 - g22).astype(bf16))
        m5 = tn(_cat(0, o11 + o12, ora), wo_v[256:D, 256:512])
        c12 = xa[:, 256:512] + m3 + m5
        m1 = tn(o11 + o22, (g11 + g22).astype(bf16))
        p11 = xa[:, 0:256] + m1 - m5
        p22 = xb[:, 256:512] + m1 + m3
        a4 = xa[:, 512:D] + tn(oa, wo_v[:, 512:D])
        m4 = tn(o22, (g21 - g11).astype(bf16))
        p11 = p11 + m4
        c11 = p11 + tn(_cat(0, o12 - o22, ora), _cat(0, g21 + g22, gr).astype(bf16))
        h_a = _cat(1, c11, c12, a4)
        b4 = xb[:, 512:D] + tn(ob, wo_v[:, 512:D])
        m2 = tn(_cat(0, o21 + o22, orb), _cat(0, wo_v[0:256, 0:256], wo_v[512:D, 0:256]))
        c21 = xb[:, 0:256] + m4 + m2
        p22 = p22 - m2
        c22 = p22 + tn(_cat(0, o21 - o11, orb), _cat(0, g11 + g12, gr).astype(bf16))
        h_b = _cat(1, c21, c22, b4)
        hs = [(h_a, _layernorm(h_a)), (h_b, _layernorm(h_b))]

        ha, hb = hs[0][1], hs[1][1]
        a11, a12, a21, a22 = ha[:, 0:256], ha[:, 256:512], hb[:, 0:256], hb[:, 256:512]
        ra, rb = ha[:, 512:D], hb[:, 512:D]
        s1, s2r, s3, s4, s5r, s6r, s7r = [v.astype(bf16) for v in (
            a11 + a22, _cat(1, a21 + a22, rb), a11, a22, _cat(1, a11 + a12, ra), _cat(1, a21 - a11, rb),
            _cat(1, a12 - a22, ra))]

        def wcols(r0, r1, c0):
            return _cat(1, wg_v[r0:r1, c0:c0 + CW], wu_v[r0:r1, c0:c0 + CW])

        def wcols32(r0, r1, c0):
            return _cat(1, wg_v[r0:r1, c0:c0 + CW].astype(f32), wu_v[r0:r1, c0:c0 + CW].astype(f32))

        def glu(c):
            return jax.nn.gelu(c[:, 0:CW], approximate=True) * c[:, CW:2 * CW]

        m5s = [_mm(s5r, wcols(256, D, HF + c * CW)) for c in range(NA)]
        for c in range(NCH):
            c1, c2 = c * CW, HF + c * CW
            f11, f12, f21, f22 = wcols32(0, 256, c1), wcols32(0, 256, c2), wcols32(256, 512, c1), wcols32(256, 512, c2)
            r12 = wcols32(512, D, c1) + wcols32(512, D, c2)
            m5 = m5s[c] if c < NA else _mm(s5r, wcols(256, D, c2))
            m2 = _mm(s2r, _cat(0, wcols(0, 256, c1), wcols(512, D, c1)))
            m1 = _mm(s1, (f11 + f22).astype(bf16))
            p22 = m1 - m2
            p11 = m1 - m5
            m3 = _mm(s3, (f12 - f22).astype(bf16))
            c12 = m3 + m5
            p22 = p22 + m3
            m4 = _mm(s4, (f21 - f11).astype(bf16))
            c21 = m2 + m4
            p11 = p11 + m4
            c11 = p11 + _mm(s7r, _cat(0, f21 + f22, r12).astype(bf16))
            c22 = p22 + _mm(s6r, _cat(0, f11 + f12, r12).astype(bf16))
            q11, q12, q21, q22 = glu(c11), glu(c12), glu(c21), glu(c22)
            for k, v in enumerate((q11 + q22, q21 + q22, q11, q22, q11 + q12, q21 - q11, q12 - q22, q12, q21)):
                d_s[:, k * HF + c * CW:k * HF + (c + 1) * CW] = _pk(v.astype(bf16))

        def dn_rhs(k0, k1):
            f11, f12 = wd_v[k0:k1, 0:256].astype(f32), wd_v[k0:k1, 256:512].astype(f32)
            f21, f22 = wd_v[HF + k0:HF + k1, 0:256].astype(f32), wd_v[HF + k0:HF + k1, 256:512].astype(f32)
            w4 = _cat(0, wd_v[k0:k1, 512:D], wd_v[HF + k0:HF + k1, 512:D])
            return [(f11 + f22).astype(bf16), wd_v[k0:k1, 0:256], (f12 - f22).astype(bf16), (f21 - f11).astype(bf16),
                    wd_v[HF + k0:HF + k1, 256:512], (f11 + f12).astype(bf16), (f21 + f22).astype(bf16), w4, w4]

        def dn_stage(ya, yb, r0, r1, k0, k1, t, done=None):
            rows = slice(r0 // 2, r1 // 2)

            def f(k):
                if k < 7:
                    return _mm(_upk(d_s[rows, k * HF + k0:k * HF + k1]), t[k])
                lo, hi = ((2, 7), (8, 3))[k - 7]
                return _mm(_upk(_cat(1, d_s[rows, lo * HF + k0:lo * HF + k1], d_s[rows, hi * HF + k0:hi * HF + k1])),
                           t[k])

            a4 = ya[:, 512:D] + f(7)
            m5, m2, m1 = f(4), f(1), f(0)
            p11 = ya[:, 0:256] + m1 - m5
            p22 = yb[:, 256:512] + m1 - m2
            m3 = f(2)
            c12 = ya[:, 256:512] + m5 + m3
            p22 = p22 + m3
            m4 = f(3)
            c21 = yb[:, 0:256] + m2 + m4
            p11 = p11 + m4
            ya = _cat(1, p11 + f(6), c12, a4)
            if done is not None:
                done(0, ya)
            b4 = yb[:, 512:D] + f(8)
            yb = _cat(1, c21, p22 + f(5), b4)
            if done is not None:
                done(1, yb)
            return ya, yb

        ya, yb = dn_stage(hs[0][0], hs[1][0], 0, SB, 0, KD, dn_rhs(0, KD))
        t = dn_rhs(KD, HF)
        r0 = 0
        for nr in CH:
            def done(s_, y):
                rows = pl.ds(off + s_ * SB + r0, nr)
                out_v[rows, :] = y.astype(bf16)
                pltpu.make_async_copy(out_v.at[rows], out_hbm.at[rows], o_sem.at[0]).start()

            dn_stage(ya[r0:r0 + nr], yb[r0:r0 + nr], r0, r0 + nr, KD, HF, t, done)
            r0 += nr
        return carry

    lax.fori_loop(0, NSUB // 2, phase2, 0)
    pltpu.make_async_copy(out_v, out_hbm, o_sem.at[0]).wait()


def _compiler_params():
    try:
        return pltpu.CompilerParams(vmem_limit_bytes=100 * 1024 * 1024, disable_bounds_checks=True,
                                    disable_semaphore_checks=True)
    except TypeError:
        return pltpu.CompilerParams(vmem_limit_bytes=100 * 1024 * 1024)


@jax.jit
def pallas_sequential_preLN__linear_kernel_hedgehog__geglu_ffn__prompt_kernel(
    A_x: jax.Array,
    A_wqkv: jax.Array,
    A_w_phi: jax.Array,
    A_wo: jax.Array,
    B_x: jax.Array,
    B_w_gate: jax.Array,
    B_w_up: jax.Array,
    B_w_down: jax.Array,
):
    x = A_x.reshape(S, D)
    wphi_t = jnp.transpose(A_w_phi, (1, 2, 0))
    anyspec = pl.BlockSpec(memory_space=pl.ANY)
    out = pl.pallas_call(
        _kernel,
        out_shape=jax.ShapeDtypeStruct((S, D), bf16),
        in_specs=[anyspec] * 7,
        out_specs=anyspec,
        scratch_shapes=[
            pltpu.VMEM((S, D), bf16),
            pltpu.VMEM((D, 3 * D), bf16),
            pltpu.VMEM((DH, DH, H), bf16),
            pltpu.VMEM((D, D), bf16),
            pltpu.VMEM((D, F), bf16),
            pltpu.VMEM((D, F), bf16),
            pltpu.VMEM((F, D), bf16),
            pltpu.VMEM((S, D), bf16),
            pltpu.SMEM((1,), jnp.int32),
            pltpu.VMEM(((SB - AR) // 2, D), u32),
            pltpu.VMEM((SB, D), u32),
            pltpu.VMEM((2 * DP + D, 2 * SB), f32),
            pltpu.VMEM((XROW + AR // 2, D), u32),
            pltpu.VMEM(((2 * DP + D) // 4, 5 * 256), u32),
            pltpu.VMEM((NG * 40, S), u32),
            pltpu.VMEM((NG * 40, 4 * SB), u32),
            pltpu.VMEM((344, 4 * SB), u32),
            pltpu.VMEM((688, 128), f32),
            pltpu.VMEM((344, 128), u32),
            pltpu.VMEM((SB // 2, 9 * HF), u32),
            pltpu.SemaphoreType.DMA((4,)),
            pltpu.SemaphoreType.DMA((8,)),
            pltpu.SemaphoreType.DMA((1,)),
        ],
        compiler_params=_compiler_params(),
    )(x, A_wqkv, wphi_t, A_wo, B_w_gate, B_w_up, B_w_down)
    return out.reshape(1, S, D)
```
